```python
import jax
import jax.numpy as jnp

def _softmax(x, axis=-1):
    return jax.nn.softmax(x, axis=axis)
def _gelu(x):
    return jax.nn.gelu(x, approximate=True)
def _silu(x):
    return jax.nn.silu(x)
def _sigmoid(x):
    return jax.nn.sigmoid(x)
def _layernorm(x, axis=-1, eps=1e-5):
    m = jnp.mean(x, axis=axis, keepdims=True)
    v = jnp.var(x, axis=axis, keepdims=True)
    return (x - m) / jnp.sqrt(v + eps)
def _scatter_add(tgt, idx, src, axis=0):
    return tgt.at[idx].add(src)
def _segment_sum(src, seg, n):
    return jax.ops.segment_sum(src, seg, n)
class _Rng:
    def __init__(self, key):
        self._k = key
    def _next(self):
        self._k, sub = jax.random.split(self._k)
        return sub
    def normal(self, shape):
        return jax.random.normal(self._next(), shape, dtype=jnp.bfloat16)
    def randint(self, lo, hi, shape):
        return jax.random.randint(self._next(), shape, lo, hi, dtype=jnp.int32)
    def uniform(self, shape, lo=0.0, hi=1.0):
        return jax.random.uniform(self._next(), shape, jnp.bfloat16, lo, hi)
    def permutation(self, n):
        return jax.random.permutation(self._next(), n)


kernel_name = 'recurrent_scan__sliding_local_dilated__glu_gated_swiglu__prompt'

def setup_inputs():
    _rng = _Rng(jax.random.key(int.from_bytes(__import__("os").urandom(4), "little")))
    _w = (lambda a: (lambda t: t.astype(jnp.bfloat16) if jnp.issubdtype(t.dtype, jnp.floating) else t)(jnp.asarray(a)))
    def _A_setup():
        B, S, D = 1, 2048, 1024
        return {
            "x": _w((lambda *s: _rng.normal(s) * 0.05)(B, S, D)),
            "wqkv": _w((lambda *s: _rng.normal(s) * 0.05)(D, 3 * D)),
            "wo": _w((lambda *s: _rng.normal(s) * 0.05)(D, D)),
        }
    _A_in = _A_setup()

    def _B_setup():
        B, S, D, F = 1, 2048, 1024, 3584
        return {
            "x": _w((lambda *s: _rng.normal(s) * 0.05)(B, S, D)),
            "w1": _w((lambda *s: _rng.normal(s) * 0.05)(D, F) * (2.0 / D) ** 0.5),
            "w3": _w((lambda *s: _rng.normal(s) * 0.05)(D, F) * (2.0 / D) ** 0.5),
            "w2": _w((lambda *s: _rng.normal(s) * 0.05)(F, D) * (2.0 / F) ** 0.5),
        }
    _B_in = _B_setup()

    return {
        "A_x": _A_in["x"],
        "A_wqkv": _A_in["wqkv"],
        "A_wo": _A_in["wo"],
        "B_x": _B_in["x"],
        "B_w1": _B_in["w1"],
        "B_w3": _B_in["w3"],
        "B_w2": _B_in["w2"],
    }

def reference(A_x, A_wqkv, A_wo, B_x, B_w1, B_w3, B_w2):
    def _A_ref(x, wqkv, wo):
        B, S, D = x.shape
        H = 32; Dh = D // H
        W, dil = 8, 2
        qkv = (lambda x, *d: x.transpose(*d))((x @ wqkv).reshape(B, S, 3, H, Dh), 2, 0, 3, 1, 4)
        q, k, v = qkv[0], qkv[1], qkv[2]
        scale = Dh ** -0.5
        pos = jnp.arange(S)
        off = jnp.arange(W) * dil
        idx = pos[:, None] - off[None, :]
        mask = idx >= 0
        idx_c = jnp.where(mask, idx, 0).reshape(-1)
        kg = k[:, :, idx_c, :].reshape(B, H, S, W, Dh)
        vg = v[:, :, idx_c, :].reshape(B, H, S, W, Dh)
        logits = jnp.einsum("bhsd,bhswd->bhsw", q, kg) * scale
        logits = jnp.where(mask[None, None, :, :], logits, -1e9)
        attn = _softmax(logits, axis=-1)
        o = jnp.einsum("bhsw,bhswd->bhsd", attn, vg)
        return (lambda x, *d: x.transpose(*d))(o, 0, 2, 1, 3).reshape(B, S, D) @ wo

    def _B_ref(x, w1, w3, w2):
        gate = jnp.einsum("bsd,df->bsf", x, w1)
        up = jnp.einsum("bsd,df->bsf", x, w3)
        h = _silu(gate) * up
        out = jnp.einsum("bsf,fd->bsd", h, w2)
        return out

    x = A_x
    xn = _layernorm(x, axis=-1)
    s = _A_ref(xn, A_wqkv, A_wo)
    g = _silu(_B_ref(xn, B_w1, B_w3, B_w2))
    return x + s * g
```

```python
import functools
import math

import jax
import jax.numpy as jnp
import jax.experimental.pallas as pl
import jax.experimental.pallas.tpu as pltpu

_H = 32
_W = 8
_DIL = 2
_HALO = 16
_BM = 256
_RG = 16
_F0 = 640
_FC = 512
_NEG = -1e9
_NA = 2


def _silu(x):
    return x * pl.reciprocal(1.0 + jnp.exp(-x), approx=True)


def _lane_exchange(blocks, lane):
    blocks = list(blocks)
    for b in range(3):
        sh = 2 << b
        m = (lane & sh) != 0
        for i in range(8):
            if i & (1 << b):
                continue
            lo, hi = blocks[i], blocks[i | (1 << b)]
            blocks[i] = jnp.where(m, pltpu.roll(hi, sh, 1), lo)
            blocks[i | (1 << b)] = jnp.where(m, hi, pltpu.roll(lo, 128 - sh, 1))
    return blocks


def _xor_add(x, lane, sh):
    m = (lane & sh) != 0
    return x + jnp.where(m, pltpu.roll(x, sh, 1), pltpu.roll(x, 128 - sh, 1))


def _kernel(x_hbm, wqkv_hbm, wo_hbm, w1_hbm, w3_hbm, w2_hbm, o_ref,
            x_s, xn_s, acc_s, wqkv_s, wo_s, w1_s, w3_s, w2_s, k_s, v_s, sem_x, sem_w,
            *, S, D, F):
    NB = S // _BM
    step = pl.program_id(0)
    f32, bf16 = jnp.float32, jnp.bfloat16

    def x_copy(r):
        rows = pl.ds(r * _BM, _BM)
        return pltpu.make_async_copy(x_hbm.at[rows, :], x_s.at[rows, :], sem_x.at[r])

    def w_copies_first():
        c = pl.ds(0, _F0)
        return [
            pltpu.make_async_copy(w1_hbm.at[:, c], w1_s.at[:, c], sem_w.at[0]),
            pltpu.make_async_copy(w3_hbm.at[:, c], w3_s.at[:, c], sem_w.at[1]),
            pltpu.make_async_copy(w2_hbm.at[c, :], w2_s.at[c, :], sem_w.at[2]),
        ]

    def w_copies_rest():
        c = pl.ds(_F0, F - _F0)
        return [
            pltpu.make_async_copy(wqkv_hbm, wqkv_s, sem_w.at[3]),
            pltpu.make_async_copy(w1_hbm.at[:, c], w1_s.at[:, c], sem_w.at[4]),
            pltpu.make_async_copy(w3_hbm.at[:, c], w3_s.at[:, c], sem_w.at[5]),
            pltpu.make_async_copy(w2_hbm.at[c, :], w2_s.at[c, :], sem_w.at[6]),
            pltpu.make_async_copy(wo_hbm, wo_s, sem_w.at[7]),
        ]

    @pl.when(step == 0)
    def _():
        x_copy(0).start()
        for c in w_copies_first():
            c.start()
        for r in range(1, NB):
            x_copy(r).start()
        for c in w_copies_rest():
            c.start()
        k_s[:, pl.ds(0, _HALO), :] = jnp.zeros((8, _HALO, 128), f32)
        v_s[:, pl.ds(0, _HALO), :] = jnp.zeros((8, _HALO, 128), f32)
        for c in w_copies_first():
            c.wait()

    def ffn_chunk(xn, c0, cn):
        cols = pl.ds(c0, cn)
        g = jnp.dot(xn, w1_s[:, cols], preferred_element_type=f32)
        u = jnp.dot(xn, w3_s[:, cols], preferred_element_type=f32)
        h = (_silu(g) * u).astype(bf16)
        return jnp.dot(h, w2_s[cols, :], preferred_element_type=f32)

    @pl.when(step < NB)
    def _():
        x_copy(step).wait()
        rows = pl.ds(pl.multiple_of(step * _BM, _BM), _BM)
        x = x_s[rows, :].astype(f32)
        mean = jnp.mean(x, axis=-1, keepdims=True)
        xc = x - mean
        var = jnp.mean(xc * xc, axis=-1, keepdims=True)
        xn = (xc * jax.lax.rsqrt(var + 1e-5)).astype(bf16)
        xn_s[rows, :] = xn
        acc_s[rows, :] = ffn_chunk(xn, 0, _F0)

    @pl.when(step >= NB)
    def _():
        blk = step - NB

        @pl.when(blk == 0)
        def _():
            for c in w_copies_rest():
                c.wait()

        rows = pl.ds(pl.multiple_of(blk * _BM, _BM), _BM)
        xn = xn_s[rows, :]
        lane = jax.lax.broadcasted_iota(jnp.int32, (_RG, 128), 1)

        def proj(c0):
            return jnp.dot(xn, wqkv_s[:, pl.ds(c0, D)], preferred_element_type=f32)

        def groups(y):
            for g in range(_BM // _RG):
                yg = y[g * _RG:(g + 1) * _RG, :]
                yield g, _lane_exchange(
                    [yg[:, j * 128:(j + 1) * 128] for j in range(8)], lane)

        for src, dst in ((1, k_s), (2, v_s)):
            for g, blocks in groups(proj(src * D)):
                for j in range(8):
                    dst[j, pl.ds(_HALO + g * _RG, _RG), :] = blocks[j]

        chunks = []
        c0 = _F0
        while c0 < F:
            cn = min(_FC, F - c0)
            chunks.append((c0, cn))
            c0 += cn
        n_groups = _BM // _RG

        scale = (D // _H) ** -0.5
        c_exp = scale * math.log2(math.e)
        o_groups = []
        qproj = proj(0)
        acc = acc_s[rows, :]
        for c0, cn in chunks[:_NA]:
            acc = acc + ffn_chunk(xn, c0, cn)
        for g, q in groups(qproj):
            r0 = _HALO + g * _RG
            masked = g * _RG < (_W - 1) * _DIL
            if masked:
                grow = (jax.lax.broadcasted_iota(jnp.int32, (_RG, 128), 0)
                        + (blk * _BM + g * _RG))
            logits = []
            for w in range(_W):
                kr = pl.ds(r0 - _DIL * w, _RG)
                l = q[0] * k_s[0, kr, :]
                for j in range(1, 8):
                    l = l + q[j] * k_s[j, kr, :]
                l = _xor_add(l, lane, 16)
                l = _xor_add(l, lane, 1)
                if masked and w > 0:
                    l = jnp.where(grow >= _DIL * w, l, _NEG / scale)
                logits.append(l)
            m = functools.reduce(jnp.maximum, logits)
            e = [jnp.exp2((l - m) * c_exp) for l in logits]
            inv = pl.reciprocal(functools.reduce(jnp.add, e), approx=True)
            p = [ei * inv for ei in e]
            ob = []
            for j in range(8):
                if masked:
                    v0 = jnp.broadcast_to(v_s[j, pl.ds(_HALO, 1), :], (_RG, 128))
                oj = None
                for w in range(_W):
                    vw = v_s[j, pl.ds(r0 - _DIL * w, _RG), :]
                    if masked and w > 0:
                        vw = jnp.where(grow >= _DIL * w, vw, v0)
                    t = p[w] * vw
                    oj = t if oj is None else oj + t
                ob.append(oj)
            ob = _lane_exchange(ob, lane)
            o_groups.append(jnp.concatenate(ob, axis=1).astype(bf16))
        o = jnp.concatenate(o_groups, axis=0)

        k_s[:, pl.ds(0, _HALO), :] = k_s[:, pl.ds(_BM, _HALO), :]
        v_s[:, pl.ds(0, _HALO), :] = v_s[:, pl.ds(_BM, _HALO), :]

        s = jnp.dot(o, wo_s[...], preferred_element_type=f32)

        for c0, cn in chunks[_NA:]:
            acc = acc + ffn_chunk(xn, c0, cn)

        o_ref[...] = (x_s[rows, :].astype(f32) + s * _silu(acc)).astype(o_ref.dtype)


@jax.jit
def pallas_recurrent_scan__sliding_local_dilated__glu_gated_swiglu__prompt_kernel(
    A_x: jax.Array,
    A_wqkv: jax.Array,
    A_wo: jax.Array,
    B_x: jax.Array,
    B_w1: jax.Array,
    B_w3: jax.Array,
    B_w2: jax.Array,
):
    del B_x
    B, S0, D = A_x.shape
    F = B_w1.shape[1]
    S = B * S0
    assert B == 1 and D == 1024 and S % _BM == 0
    NB = S // _BM
    x = A_x.reshape(S, D)
    f32, bf16 = jnp.float32, jnp.bfloat16
    any_spec = pl.BlockSpec(memory_space=pl.ANY)
    out = pl.pallas_call(
        functools.partial(_kernel, S=S, D=D, F=F),
        grid=(2 * NB,),
        in_specs=[any_spec] * 6,
        out_specs=pl.BlockSpec((_BM, D), lambda i: (jnp.maximum(i - NB, 0), 0)),
        out_shape=jax.ShapeDtypeStruct((S, D), A_x.dtype),
        scratch_shapes=[
            pltpu.VMEM((S, D), bf16),
            pltpu.VMEM((S, D), bf16),
            pltpu.VMEM((S, D), f32),
            pltpu.VMEM((D, 3 * D), bf16),
            pltpu.VMEM((D, D), bf16),
            pltpu.VMEM((D, F), bf16),
            pltpu.VMEM((D, F), bf16),
            pltpu.VMEM((F, D), bf16),
            pltpu.VMEM((8, _HALO + _BM, 128), f32),
            pltpu.VMEM((8, _HALO + _BM, 128), f32),
            pltpu.SemaphoreType.DMA((NB,)),
            pltpu.SemaphoreType.DMA((8,)),
        ],
        compiler_params=pltpu.CompilerParams(
            dimension_semantics=("arbitrary",),
            vmem_limit_bytes=100 * 1024 * 1024,
        ),
    )(x, A_wqkv, A_wo, B_w1, B_w3, B_w2)
    return out.reshape(B, S0, D)
```

```python
import functools
import math

import jax
import jax.numpy as jnp
import jax.experimental.pallas as pl
import jax.experimental.pallas.tpu as pltpu

_H = 32
_W = 8
_DIL = 2
_HALO = 16
_BM = 256
_RG = 16
_F0 = 640
_FC = 512
_NEG = -1e9
_NA = 3
_DEPTH = 1


def _silu(x):
    return x * pl.reciprocal(1.0 + jnp.exp(-x), approx=True)


def _lane_exchange(blocks, lane):
    blocks = list(blocks)
    for b in range(3):
        sh = 2 << b
        m = (lane & sh) != 0
        for i in range(8):
            if i & (1 << b):
                continue
            lo, hi = blocks[i], blocks[i | (1 << b)]
            blocks[i] = jnp.where(m, pltpu.roll(hi, sh, 1), lo)
            blocks[i | (1 << b)] = jnp.where(m, hi, pltpu.roll(lo, 128 - sh, 1))
    return blocks


def _xor_add(x, lane, sh):
    m = (lane & sh) != 0
    return x + jnp.where(m, pltpu.roll(x, sh, 1), pltpu.roll(x, 128 - sh, 1))


def _kernel(x_hbm, wqkv_hbm, wo_hbm, w1_hbm, w3_hbm, w2_hbm, o_ref,
            x_s, xn_s, acc_s, wqkv_s, wo_s, w1_s, w3_s, w2_s, att_s, sem_x, sem_w,
            *, S, D, F):
    NB = S // _BM
    step = pl.program_id(0)
    f32, bf16 = jnp.float32, jnp.bfloat16

    def b16(ref):
        return ref.bitcast(bf16)

    def ld(ref, rows, cols=slice(None)):
        st = rows.start // 2 if isinstance(rows.start, int) else pl.multiple_of(rows.start // 2, 8)
        return pltpu.bitcast(ref[pl.ds(st, rows.size // 2), cols], bf16)

    def x_copy(r):
        rows = pl.ds(r * _BM, _BM)
        return pltpu.make_async_copy(x_hbm.at[rows, :], b16(x_s).at[rows, :], sem_x.at[r])

    def w_copies_first():
        c = pl.ds(0, _F0)
        return [
            pltpu.make_async_copy(w1_hbm.at[:, c], b16(w1_s).at[:, c], sem_w.at[0]),
            pltpu.make_async_copy(w3_hbm.at[:, c], b16(w3_s).at[:, c], sem_w.at[1]),
            pltpu.make_async_copy(w2_hbm.at[c, :], b16(w2_s).at[c, :], sem_w.at[2]),
        ]

    def w_copies_rest():
        c = pl.ds(_F0, F - _F0)
        return [
            pltpu.make_async_copy(wqkv_hbm, b16(wqkv_s), sem_w.at[3]),
            pltpu.make_async_copy(w1_hbm.at[:, c], b16(w1_s).at[:, c], sem_w.at[4]),
            pltpu.make_async_copy(w3_hbm.at[:, c], b16(w3_s).at[:, c], sem_w.at[5]),
            pltpu.make_async_copy(w2_hbm.at[c, :], b16(w2_s).at[c, :], sem_w.at[6]),
            pltpu.make_async_copy(wo_hbm, b16(wo_s), sem_w.at[7]),
        ]

    def layernorm(r):
        rows = pl.ds(pl.multiple_of(r * _BM, _BM), _BM)
        x = ld(x_s, rows).astype(f32)
        mean = jnp.mean(x, axis=-1, keepdims=True)
        xc = x - mean
        var = jnp.mean(xc * xc, axis=-1, keepdims=True)
        xn = (xc * jax.lax.rsqrt(var + 1e-5)).astype(bf16)
        xn_s[pl.ds(pl.multiple_of(r * (_BM // 2), 8), _BM // 2), :] = pltpu.bitcast(xn, jnp.uint32)

    @pl.when(step == 0)
    def _():
        x_copy(0).start()
        for c in w_copies_first():
            c.start()
        for r in range(1, NB):
            x_copy(r).start()
        for c in w_copies_rest():
            c.start()
        att_s[pl.ds(0, 2), :, pl.ds(0, _HALO), :] = jnp.zeros((2, 8, _HALO, 128), f32)
        x_copy(0).wait()
        layernorm(0)
        for c in w_copies_first():
            c.wait()

    def ffn_chunk(xn, c0, cn):
        cols = pl.ds(c0, cn)
        g = jnp.dot(xn, ld(w1_s, pl.ds(0, D), cols), preferred_element_type=f32)
        u = jnp.dot(xn, ld(w3_s, pl.ds(0, D), cols), preferred_element_type=f32)
        h = (_silu(g) * u).astype(bf16)
        return jnp.dot(h, ld(w2_s, cols), preferred_element_type=f32)

    @pl.when(step < NB)
    def _():
        nxt = jnp.minimum(step + 1, NB - 1)

        @pl.when(step + 1 < NB)
        def _():
            x_copy(nxt).wait()

        rows = pl.ds(pl.multiple_of(step * _BM, _BM), _BM)
        xn = ld(xn_s, rows)
        layernorm(nxt)
        acc_s[rows, :] = ffn_chunk(xn, 0, _F0)

    @pl.when(step >= NB)
    def _():
        blk = step - NB

        @pl.when(blk == 0)
        def _():
            for c in w_copies_rest():
                c.wait()

        rows = pl.ds(pl.multiple_of(blk * _BM, _BM), _BM)
        xn = ld(xn_s, rows)
        lane = jax.lax.broadcasted_iota(jnp.int32, (_RG, 128), 1)

        def proj(c0):
            return jnp.dot(xn, ld(wqkv_s, pl.ds(0, D), pl.ds(c0, D)), preferred_element_type=f32)

        def groups(y):
            for g in range(_BM // _RG):
                yg = y[g * _RG:(g + 1) * _RG, :]
                yield g, _lane_exchange(
                    [yg[:, j * 128:(j + 1) * 128] for j in range(8)], lane)

        K, V, Q, O = 0, 1, 2, 3
        for src, dst in ((1, K), (2, V), (0, Q)):
            for g, blocks in groups(proj(src * D)):
                for j in range(8):
                    att_s[dst, j, pl.ds(_HALO + g * _RG, _RG), :] = blocks[j]

        chunks = []
        c0 = _F0
        while c0 < F:
            cn = min(_FC, F - c0)
            chunks.append((c0, cn))
            c0 += cn

        acc = acc_s[rows, :]
        for c0, cn in chunks[:_NA]:
            acc = acc + ffn_chunk(xn, c0, cn)

        scale = (D // _H) ** -0.5
        c_exp = scale * math.log2(math.e)
        zero = pl.multiple_of(jnp.minimum(blk, 0), 8)

        def grow(g):
            return (jax.lax.broadcasted_iota(jnp.int32, (_RG, 128), 0)
                    + (blk * _BM + g * _RG))

        def logits_of(g):
            r0 = _HALO + g * _RG
            masked = g * _RG < (_W - 1) * _DIL
            q = [att_s[Q, j, pl.ds(r0, _RG), :] for j in range(8)]
            logits = []
            for w in range(_W):
                kr = pl.ds(r0 - _DIL * w, _RG)
                l = q[0] * att_s[K, 0, kr, :]
                for j in range(1, 8):
                    l = l + q[j] * att_s[K, j, kr, :]
                l = _xor_add(l, lane, 16)
                l = _xor_add(l, lane, 1)
                if masked and w > 0:
                    l = jnp.where(grow(g) >= _DIL * w, l, _NEG / scale)
                logits.append(l)
            m = functools.reduce(jnp.maximum, logits)
            e = [jnp.exp2((l - m) * c_exp) for l in logits]
            inv = pl.reciprocal(functools.reduce(jnp.add, e), approx=True)
            return [ei * inv for ei in e]

        def mix_v(g, p):
            r0 = _HALO + g * _RG
            masked = g * _RG < (_W - 1) * _DIL
            ob = []
            for j in range(8):
                if masked:
                    v0 = jnp.broadcast_to(att_s[V, j, pl.ds(_HALO, 1), :], (_RG, 128))
                oj = None
                for w in range(_W):
                    vw = att_s[V, j, pl.ds(r0 - _DIL * w, _RG), :]
                    if masked and w > 0:
                        vw = jnp.where(grow(g) >= _DIL * w, vw, v0)
                    t = p[w] * vw
                    oj = t if oj is None else oj + t
                ob.append(oj)
            return _lane_exchange(ob, lane)

        n_groups = _BM // _RG
        pending = []
        for g in range(n_groups):
            pending.append((g, mix_v(g, logits_of(g))))
            if len(pending) > _DEPTH - 1:
                gg, ob = pending.pop(0)
                for j in range(8):
                    att_s[O, j, pl.ds(zero + gg * _RG, _RG), :] = ob[j]
        for gg, ob in pending:
            for j in range(8):
                att_s[O, j, pl.ds(zero + gg * _RG, _RG), :] = ob[j]

        o = jnp.concatenate(
            [att_s[O, j, pl.ds(0, _BM), :] for j in range(8)], axis=1).astype(bf16)

        for t in (K, V):
            att_s[t, :, pl.ds(0, _HALO), :] = att_s[t, :, pl.ds(_BM, _HALO), :]

        s = jnp.dot(o, ld(wo_s, pl.ds(0, D)), preferred_element_type=f32)

        for c0, cn in chunks[_NA:]:
            acc = acc + ffn_chunk(xn, c0, cn)

        o_ref[...] = (ld(x_s, rows).astype(f32) + s * _silu(acc)).astype(o_ref.dtype)


@jax.jit
def pallas_recurrent_scan__sliding_local_dilated__glu_gated_swiglu__prompt_kernel(
    A_x: jax.Array,
    A_wqkv: jax.Array,
    A_wo: jax.Array,
    B_x: jax.Array,
    B_w1: jax.Array,
    B_w3: jax.Array,
    B_w2: jax.Array,
):
    del B_x
    B, S0, D = A_x.shape
    F = B_w1.shape[1]
    S = B * S0
    assert B == 1 and D == 1024 and S % _BM == 0
    NB = S // _BM
    x = A_x.reshape(S, D)
    f32, u32 = jnp.float32, jnp.uint32
    any_spec = pl.BlockSpec(memory_space=pl.ANY)
    out = pl.pallas_call(
        functools.partial(_kernel, S=S, D=D, F=F),
        grid=(2 * NB,),
        in_specs=[any_spec] * 6,
        out_specs=pl.BlockSpec((_BM, D), lambda i: (jnp.maximum(i - NB, 0), 0)),
        out_shape=jax.ShapeDtypeStruct((S, D), A_x.dtype),
        scratch_shapes=[
            pltpu.VMEM((S // 2, D), u32),
            pltpu.VMEM((S // 2, D), u32),
            pltpu.VMEM((S, D), f32),
            pltpu.VMEM((D // 2, 3 * D), u32),
            pltpu.VMEM((D // 2, D), u32),
            pltpu.VMEM((D // 2, F), u32),
            pltpu.VMEM((D // 2, F), u32),
            pltpu.VMEM((F // 2, D), u32),
            pltpu.VMEM((4, 8, _HALO + _BM, 128), f32),
            pltpu.SemaphoreType.DMA((NB,)),
            pltpu.SemaphoreType.DMA((8,)),
        ],
        compiler_params=pltpu.CompilerParams(
            dimension_semantics=("arbitrary",),
            vmem_limit_bytes=100 * 1024 * 1024,
        ),
    )(x, A_wqkv, A_wo, B_w1, B_w3, B_w2)
    return out.reshape(B, S0, D)
```

```python
import functools
import math

import jax
import jax.numpy as jnp
import jax.experimental.pallas as pl
import jax.experimental.pallas.tpu as pltpu

_H = 32
_W = 8
_DIL = 2
_HALO = 16
_BM = 256
_RG = 16
_F0 = 640
_FC = 512
_NEG = -1e9
_NA = 3
_DEPTH = 1


def _silu(x):
    return x * pl.reciprocal(1.0 + jnp.exp(-x), approx=True)


def _lane_exchange(blocks, lane):
    blocks = list(blocks)
    for b in range(3):
        sh = 2 << b
        m = (lane & sh) != 0
        for i in range(8):
            if i & (1 << b):
                continue
            lo, hi = blocks[i], blocks[i | (1 << b)]
            blocks[i] = jnp.where(m, pltpu.roll(hi, sh, 1), lo)
            blocks[i | (1 << b)] = jnp.where(m, hi, pltpu.roll(lo, 128 - sh, 1))
    return blocks


def _xor_add(x, lane, sh):
    m = (lane & sh) != 0
    return x + jnp.where(m, pltpu.roll(x, sh, 1), pltpu.roll(x, 128 - sh, 1))


def _kernel(x_hbm, wqkv_hbm, wo_hbm, w1_hbm, w3_hbm, w2_hbm, o_ref,
            x_s, xn_s, acc_s, wqkv_s, wo_s, w1_s, w3_s, w2_s, att_s, sem_x, sem_w,
            *, S, D, F):
    NB = S // _BM
    step = pl.program_id(0)
    f32, bf16 = jnp.float32, jnp.bfloat16

    def b16(ref):
        return ref.bitcast(bf16)

    def ld(ref, rows, cols=slice(None)):
        st = rows.start // 2 if isinstance(rows.start, int) else pl.multiple_of(rows.start // 2, 8)
        return pltpu.bitcast(ref[pl.ds(st, rows.size // 2), cols], bf16)

    def x_copy(r):
        rows = pl.ds(r * _BM, _BM)
        return pltpu.make_async_copy(x_hbm.at[rows, :], b16(x_s).at[rows, :], sem_x.at[r])

    def w_copies_first():
        c = pl.ds(0, _F0)
        return [
            pltpu.make_async_copy(w1_hbm.at[:, c], b16(w1_s).at[:, c], sem_w.at[0]),
            pltpu.make_async_copy(w3_hbm.at[:, c], b16(w3_s).at[:, c], sem_w.at[1]),
            pltpu.make_async_copy(w2_hbm.at[c, :], b16(w2_s).at[c, :], sem_w.at[2]),
        ]

    def w_copies_rest():
        c = pl.ds(_F0, F - _F0)
        return [
            pltpu.make_async_copy(wqkv_hbm, b16(wqkv_s), sem_w.at[3]),
            pltpu.make_async_copy(w1_hbm.at[:, c], b16(w1_s).at[:, c], sem_w.at[4]),
            pltpu.make_async_copy(w3_hbm.at[:, c], b16(w3_s).at[:, c], sem_w.at[5]),
            pltpu.make_async_copy(w2_hbm.at[c, :], b16(w2_s).at[c, :], sem_w.at[6]),
            pltpu.make_async_copy(wo_hbm, b16(wo_s), sem_w.at[7]),
        ]

    def layernorm(r):
        rows = pl.ds(pl.multiple_of(r * _BM, _BM), _BM)
        x = ld(x_s, rows).astype(f32)
        mean = jnp.mean(x, axis=-1, keepdims=True)
        xc = x - mean
        var = jnp.mean(xc * xc, axis=-1, keepdims=True)
        xn = (xc * jax.lax.rsqrt(var + 1e-5)).astype(bf16)
        xn_s[pl.ds(pl.multiple_of(r * (_BM // 2), 8), _BM // 2), :] = pltpu.bitcast(xn, jnp.uint32)

    def ffn_chunk(xn, c0, cn, before=(None, None, None)):
        cols = pl.ds(c0, cn)

        def wait(i):
            if before[i] is not None:
                before[i].wait()

        wait(0)
        g = jnp.dot(xn, ld(w1_s, pl.ds(0, D), cols), preferred_element_type=f32)
        wait(1)
        u = jnp.dot(xn, ld(w3_s, pl.ds(0, D), cols), preferred_element_type=f32)
        h = (_silu(g) * u).astype(bf16)
        wait(2)
        return jnp.dot(h, ld(w2_s, cols), preferred_element_type=f32)

    @pl.when(step == 0)
    def _():
        x_copy(0).start()
        for c in w_copies_first():
            c.start()
        for r in range(1, NB):
            x_copy(r).start()
        for c in w_copies_rest():
            c.start()
        att_s[pl.ds(0, 2), :, pl.ds(0, _HALO), :] = jnp.zeros((2, 8, _HALO, 128), f32)
        x_copy(0).wait()
        layernorm(0)
        rows = pl.ds(0, _BM)
        acc_s[rows, :] = ffn_chunk(ld(xn_s, rows), 0, _F0, w_copies_first())
        x_copy(1).wait()
        layernorm(1)

    @pl.when(jnp.logical_and(step > 0, step < NB))
    def _():
        nxt = jnp.minimum(step + 1, NB - 1)

        @pl.when(step + 1 < NB)
        def _():
            x_copy(nxt).wait()

        rows = pl.ds(pl.multiple_of(step * _BM, _BM), _BM)
        xn = ld(xn_s, rows)
        layernorm(nxt)
        acc_s[rows, :] = ffn_chunk(xn, 0, _F0)

    @pl.when(step >= NB)
    def _():
        blk = step - NB

        @pl.when(blk == 0)
        def _():
            for c in w_copies_rest():
                c.wait()

        rows = pl.ds(pl.multiple_of(blk * _BM, _BM), _BM)
        xn = ld(xn_s, rows)
        lane = jax.lax.broadcasted_iota(jnp.int32, (_RG, 128), 1)

        def proj(c0):
            return jnp.dot(xn, ld(wqkv_s, pl.ds(0, D), pl.ds(c0, D)), preferred_element_type=f32)

        def groups(y):
            for g in range(_BM // _RG):
                yg = y[g * _RG:(g + 1) * _RG, :]
                yield g, _lane_exchange(
                    [yg[:, j * 128:(j + 1) * 128] for j in range(8)], lane)

        K, V, Q, O = 0, 1, 2, 3
        for src, dst in ((1, K), (2, V), (0, Q)):
            for g, blocks in groups(proj(src * D)):
                for j in range(8):
                    att_s[dst, j, pl.ds(_HALO + g * _RG, _RG), :] = blocks[j]

        chunks = []
        c0 = _F0
        while c0 < F:
            cn = min(_FC, F - c0)
            chunks.append((c0, cn))
            c0 += cn

        acc = acc_s[rows, :]
        for c0, cn in chunks[:_NA]:
            acc = acc + ffn_chunk(xn, c0, cn)

        scale = (D // _H) ** -0.5
        c_exp = scale * math.log2(math.e)
        zero = pl.multiple_of(jnp.minimum(blk, 0), 8)

        def grow(g):
            return (jax.lax.broadcasted_iota(jnp.int32, (_RG, 128), 0)
                    + (blk * _BM + g * _RG))

        def logits_of(g):
            r0 = _HALO + g * _RG
            masked = g * _RG < (_W - 1) * _DIL
            logits = [None] * _W
            for j in range(8):
                q = att_s[Q, j, pl.ds(r0, _RG), :]
                for w in range(_W):
                    t = q * att_s[K, j, pl.ds(r0 - _DIL * w, _RG), :]
                    logits[w] = t if j == 0 else logits[w] + t
            for w in range(_W):
                l = _xor_add(logits[w], lane, 16)
                l = _xor_add(l, lane, 1)
                if masked and w > 0:
                    l = jnp.where(grow(g) >= _DIL * w, l, _NEG / scale)
                logits[w] = l
            m = functools.reduce(jnp.maximum, logits)
            e = [jnp.exp2((l - m) * c_exp) for l in logits]
            inv = pl.reciprocal(functools.reduce(jnp.add, e), approx=True)
            return [ei * inv for ei in e]

        def mix_v(g, p):
            r0 = _HALO + g * _RG
            masked = g * _RG < (_W - 1) * _DIL
            ob = []
            for j in range(8):
                if masked:
                    v0 = jnp.broadcast_to(att_s[V, j, pl.ds(_HALO, 1), :], (_RG, 128))
                oj = None
                for w in range(_W):
                    vw = att_s[V, j, pl.ds(r0 - _DIL * w, _RG), :]
                    if masked and w > 0:
                        vw = jnp.where(grow(g) >= _DIL * w, vw, v0)
                    t = p[w] * vw
                    oj = t if oj is None else oj + t
                ob.append(oj)
            return _lane_exchange(ob, lane)

        n_groups = _BM // _RG
        pending = []
        for g in range(n_groups):
            pending.append((g, mix_v(g, logits_of(g))))
            if len(pending) > _DEPTH - 1:
                gg, ob = pending.pop(0)
                for j in range(8):
                    att_s[O, j, pl.ds(zero + gg * _RG, _RG), :] = ob[j]
        for gg, ob in pending:
            for j in range(8):
                att_s[O, j, pl.ds(zero + gg * _RG, _RG), :] = ob[j]

        o = jnp.concatenate(
            [att_s[O, j, pl.ds(0, _BM), :] for j in range(8)], axis=1).astype(bf16)

        for t in (K, V):
            att_s[t, :, pl.ds(0, _HALO), :] = att_s[t, :, pl.ds(_BM, _HALO), :]

        s = jnp.dot(o, ld(wo_s, pl.ds(0, D)), preferred_element_type=f32)

        for c0, cn in chunks[_NA:]:
            acc = acc + ffn_chunk(xn, c0, cn)

        o_ref[...] = (ld(x_s, rows).astype(f32) + s * _silu(acc)).astype(o_ref.dtype)


@jax.jit
def pallas_recurrent_scan__sliding_local_dilated__glu_gated_swiglu__prompt_kernel(
    A_x: jax.Array,
    A_wqkv: jax.Array,
    A_wo: jax.Array,
    B_x: jax.Array,
    B_w1: jax.Array,
    B_w3: jax.Array,
    B_w2: jax.Array,
):
    del B_x
    B, S0, D = A_x.shape
    F = B_w1.shape[1]
    S = B * S0
    assert B == 1 and D == 1024 and S % _BM == 0
    NB = S // _BM
    x = A_x.reshape(S, D)
    f32, u32 = jnp.float32, jnp.uint32
    any_spec = pl.BlockSpec(memory_space=pl.ANY)
    out = pl.pallas_call(
        functools.partial(_kernel, S=S, D=D, F=F),
        grid=(2 * NB,),
        in_specs=[any_spec] * 6,
        out_specs=pl.BlockSpec((_BM, D), lambda i: (jnp.maximum(i - NB, 0), 0)),
        out_shape=jax.ShapeDtypeStruct((S, D), A_x.dtype),
        scratch_shapes=[
            pltpu.VMEM((S // 2, D), u32),
            pltpu.VMEM((S // 2, D), u32),
            pltpu.VMEM((S, D), f32),
            pltpu.VMEM((D // 2, 3 * D), u32),
            pltpu.VMEM((D // 2, D), u32),
            pltpu.VMEM((D // 2, F), u32),
            pltpu.VMEM((D // 2, F), u32),
            pltpu.VMEM((F // 2, D), u32),
            pltpu.VMEM((4, 8, _HALO + _BM, 128), f32),
            pltpu.SemaphoreType.DMA((NB,)),
            pltpu.SemaphoreType.DMA((8,)),
        ],
        compiler_params=pltpu.CompilerParams(
            dimension_semantics=("arbitrary",),
            flags={"XLA_TPU_EVENLY_DISTRIBUTE_CRITICAL_NODES": True},
            vmem_limit_bytes=100 * 1024 * 1024,
        ),
    )(x, A_wqkv, A_wo, B_w1, B_w3, B_w2)
    return out.reshape(B, S0, D)
```

```python
import functools
import math

import jax
import jax.numpy as jnp
import jax.experimental.pallas as pl
import jax.experimental.pallas.tpu as pltpu

_H = 32
_W = 8
_DIL = 2
_HALO = 16
_BM = 256
_RG = 16
_F0 = 640
_FC = 512
_NEG = -1e9
_NA = 4
_TREE = 0
_GATES = 5
_JOUTER = 0
_NORMLATE = 1
_PACKO = 0
_PORDER = "qkv"


def _silu(x):
    return x * pl.reciprocal(1.0 + jnp.exp(-x), approx=True)


def _lane_exchange(blocks, lane):
    blocks = list(blocks)
    for b in range(3):
        sh = 2 << b
        m = (lane & sh) != 0
        for i in range(8):
            if i & (1 << b):
                continue
            lo, hi = blocks[i], blocks[i | (1 << b)]
            blocks[i] = jnp.where(m, pltpu.roll(hi, sh, 1), lo)
            blocks[i | (1 << b)] = jnp.where(m, hi, pltpu.roll(lo, 128 - sh, 1))
    return blocks


def _tree(fn, xs):
    xs = list(xs)
    while len(xs) > 1:
        xs = [fn(a, b) for a, b in zip(xs[0::2], xs[1::2])] + xs[len(xs) & ~1:]
    return xs[0]


def _xor_add(x, lane, sh):
    m = (lane & sh) != 0
    return x + jnp.where(m, pltpu.roll(x, sh, 1), pltpu.roll(x, 128 - sh, 1))


def _kernel(x_hbm, wqkv_hbm, wo_hbm, w1_hbm, w3_hbm, w2_hbm, o_ref,
            x_s, xn_s, acc_s, wqkv_s, wo_s, w1_s, w3_s, w2_s, att_s, sem_x, sem_w,
            *, S, D, F):
    NB = S // _BM
    step = pl.program_id(0)
    f32, bf16 = jnp.float32, jnp.bfloat16

    def b16(ref):
        return ref.bitcast(bf16)

    def ld(ref, rows, cols=slice(None)):
        st = rows.start // 2 if isinstance(rows.start, int) else pl.multiple_of(rows.start // 2, 8)
        return pltpu.bitcast(ref[pl.ds(st, rows.size // 2), cols], bf16)

    def x_copy(r):
        rows = pl.ds(r * _BM, _BM)
        return pltpu.make_async_copy(x_hbm.at[rows, :], b16(x_s).at[rows, :], sem_x.at[r])

    def w_copies_first():
        c = pl.ds(0, _F0)
        return [
            pltpu.make_async_copy(w1_hbm.at[:, c], b16(w1_s).at[:, c], sem_w.at[0]),
            pltpu.make_async_copy(w3_hbm.at[:, c], b16(w3_s).at[:, c], sem_w.at[1]),
            pltpu.make_async_copy(w2_hbm.at[c, :], b16(w2_s).at[c, :], sem_w.at[2]),
        ]

    def w_copies_rest():
        c = pl.ds(_F0, F - _F0)
        return [
            pltpu.make_async_copy(wqkv_hbm, b16(wqkv_s), sem_w.at[3]),
            pltpu.make_async_copy(w1_hbm.at[:, c], b16(w1_s).at[:, c], sem_w.at[4]),
            pltpu.make_async_copy(w3_hbm.at[:, c], b16(w3_s).at[:, c], sem_w.at[5]),
            pltpu.make_async_copy(w2_hbm.at[c, :], b16(w2_s).at[c, :], sem_w.at[6]),
            pltpu.make_async_copy(wo_hbm, b16(wo_s), sem_w.at[7]),
        ]

    def layernorm(r):
        rows = pl.ds(pl.multiple_of(r * _BM, _BM), _BM)
        x = ld(x_s, rows).astype(f32)
        mean = jnp.mean(x, axis=-1, keepdims=True)
        xc = x - mean
        var = jnp.mean(xc * xc, axis=-1, keepdims=True)
        xn = (xc * jax.lax.rsqrt(var + 1e-5)).astype(bf16)
        xn_s[pl.ds(pl.multiple_of(r * (_BM // 2), 8), _BM // 2), :] = pltpu.bitcast(xn, jnp.uint32)

    def ffn_chunk(xn, c0, cn, before=(None, None, None)):
        cols = pl.ds(c0, cn)

        def wait(i):
            if before[i] is not None:
                before[i].wait()

        wait(0)
        g = jnp.dot(xn, ld(w1_s, pl.ds(0, D), cols), preferred_element_type=f32)
        wait(1)
        u = jnp.dot(xn, ld(w3_s, pl.ds(0, D), cols), preferred_element_type=f32)
        h = (_silu(g) * u).astype(bf16)
        wait(2)
        return jnp.dot(h, ld(w2_s, cols), preferred_element_type=f32)

    @pl.when(step == 0)
    def _():
        x_copy(0).start()
        for c in w_copies_first():
            c.start()
        for r in range(1, NB):
            x_copy(r).start()
        for c in w_copies_rest():
            c.start()
        att_s[pl.ds(0, 2), :, pl.ds(0, _HALO), :] = jnp.zeros((2, 8, _HALO, 128), f32)
        x_copy(0).wait()
        layernorm(0)
        rows = pl.ds(0, _BM)
        acc_s[rows, :] = ffn_chunk(ld(xn_s, rows), 0, _F0, w_copies_first())
        x_copy(1).wait()
        layernorm(1)

    @pl.when(jnp.logical_and(step > 0, step < NB))
    def _():
        nxt = jnp.minimum(step + 1, NB - 1)

        @pl.when(step + 1 < NB)
        def _():
            x_copy(nxt).wait()

        rows = pl.ds(pl.multiple_of(step * _BM, _BM), _BM)
        xn = ld(xn_s, rows)
        layernorm(nxt)
        acc_s[rows, :] = ffn_chunk(xn, 0, _F0)

    @pl.when(step >= NB)
    def _():
        blk = step - NB

        @pl.when(blk == 0)
        def _():
            for c in w_copies_rest():
                c.wait()

        rows = pl.ds(pl.multiple_of(blk * _BM, _BM), _BM)
        xn = ld(xn_s, rows)
        lane = jax.lax.broadcasted_iota(jnp.int32, (_RG, 128), 1)

        def proj(c0):
            return jnp.dot(xn, ld(wqkv_s, pl.ds(0, D), pl.ds(c0, D)), preferred_element_type=f32)

        def groups(y):
            for g in range(_BM // _RG):
                yg = y[g * _RG:(g + 1) * _RG, :]
                yield g, _lane_exchange(
                    [yg[:, j * 128:(j + 1) * 128] for j in range(8)], lane)

        scale = (D // _H) ** -0.5
        log2e = math.log2(math.e)

        K, V, Q, O = 0, 1, 2, 3
        for name in _PORDER:
            src, dst = {"k": (1, K), "v": (2, V), "q": (0, Q)}[name]
            y = proj(src * D)
            if dst == Q:
                y = y * (scale * log2e)
            for g, blocks in groups(y):
                for j in range(8):
                    att_s[dst, j, pl.ds(_HALO + g * _RG, _RG), :] = blocks[j]

        chunks = []
        c0 = _F0
        while c0 < F:
            cn = min(_FC, F - c0)
            chunks.append((c0, cn))
            c0 += cn

        acc = acc_s[rows, :]
        for c0, cn in chunks[:_NA]:
            acc = acc + ffn_chunk(xn, c0, cn)

        zero = pl.multiple_of(jnp.minimum(blk, 0), 8)

        def grow(g):
            return (jax.lax.broadcasted_iota(jnp.int32, (_RG, 128), 0)
                    + (blk * _BM + g * _RG))

        red = _tree if _TREE else functools.reduce

        def gate(bit, val):
            if _GATES & bit:
                att_s[O, 0, pl.ds(zero + _BM, 8), :] = val[:8]

        def weights_of(g):
            r0 = _HALO + g * _RG
            masked = g * _RG < (_W - 1) * _DIL
            logits = [None] * _W

            def term(j, w, q):
                return q * att_s[K, j, pl.ds(r0 - _DIL * w, _RG), :]

            if _JOUTER:
                for j in range(8):
                    q = att_s[Q, j, pl.ds(r0, _RG), :]
                    for w in range(_W):
                        t = term(j, w, q)
                        logits[w] = t if j == 0 else logits[w] + t
            else:
                qs = [att_s[Q, j, pl.ds(r0, _RG), :] for j in range(8)]
                for w in range(_W):
                    logits[w] = functools.reduce(
                        jnp.add, [term(j, w, qs[j]) for j in range(8)])
                    if w == 3:
                        gate(1, logits[w])
                    if w in (1, 5):
                        gate(8, logits[w])
            for w in range(_W):
                l = _xor_add(logits[w], lane, 16)
                l = _xor_add(l, lane, 1)
                if masked and w > 0:
                    l = jnp.where(grow(g) >= _DIL * w, l, _NEG * log2e)
                logits[w] = l
            m = red(jnp.maximum, logits)
            e = [jnp.exp2(l - m) for l in logits]
            inv = pl.reciprocal(red(jnp.add, e), approx=True)
            gate(2, inv)
            if _NORMLATE:
                return e, inv
            return [ei * inv for ei in e], None

        def mix_v(g, p, inv):
            r0 = _HALO + g * _RG
            masked = g * _RG < (_W - 1) * _DIL
            ob = []
            for j in range(8):
                if masked:
                    v0 = jnp.broadcast_to(att_s[V, j, pl.ds(_HALO, 1), :], (_RG, 128))
                oj = None
                for w in range(_W):
                    vw = att_s[V, j, pl.ds(r0 - _DIL * w, _RG), :]
                    if masked and w > 0:
                        vw = jnp.where(grow(g) >= _DIL * w, vw, v0)
                    t = p[w] * vw
                    oj = t if oj is None else oj + t
                if inv is not None:
                    oj = oj * inv
                if j == 3:
                    gate(4, oj)
                if j in (1, 5):
                    gate(16, oj)
                if _PACKO:
                    oj = pltpu.bitcast(oj.astype(bf16), f32)
                ob.append(oj)
            if _PACKO:
                return _lane_exchange(ob, lane[:_RG // 2])
            return _lane_exchange(ob, lane)

        n_groups = _BM // _RG
        og = _RG // 2 if _PACKO else _RG
        for g in range(n_groups):
            ob = mix_v(g, *weights_of(g))
            for j in range(8):
                att_s[O, j, pl.ds(zero + g * og, og), :] = ob[j]

        o = jnp.concatenate(
            [att_s[O, j, pl.ds(0, n_groups * og), :] for j in range(8)], axis=1)
        o = pltpu.bitcast(o, bf16) if _PACKO else o.astype(bf16)

        for t in (K, V):
            att_s[t, :, pl.ds(0, _HALO), :] = att_s[t, :, pl.ds(_BM, _HALO), :]

        s = jnp.dot(o, ld(wo_s, pl.ds(0, D)), preferred_element_type=f32)

        for c0, cn in chunks[_NA:]:
            acc = acc + ffn_chunk(xn, c0, cn)

        o_ref[...] = (ld(x_s, rows).astype(f32) + s * _silu(acc)).astype(o_ref.dtype)


@jax.jit
def pallas_recurrent_scan__sliding_local_dilated__glu_gated_swiglu__prompt_kernel(
    A_x: jax.Array,
    A_wqkv: jax.Array,
    A_wo: jax.Array,
    B_x: jax.Array,
    B_w1: jax.Array,
    B_w3: jax.Array,
    B_w2: jax.Array,
):
    del B_x
    B, S0, D = A_x.shape
    F = B_w1.shape[1]
    S = B * S0
    assert B == 1 and D == 1024 and S % _BM == 0
    NB = S // _BM
    x = A_x.reshape(S, D)
    f32, u32 = jnp.float32, jnp.uint32
    any_spec = pl.BlockSpec(memory_space=pl.ANY)
    out = pl.pallas_call(
        functools.partial(_kernel, S=S, D=D, F=F),
        grid=(2 * NB,),
        in_specs=[any_spec] * 6,
        out_specs=pl.BlockSpec((_BM, D), lambda i: (jnp.maximum(i - NB, 0), 0)),
        out_shape=jax.ShapeDtypeStruct((S, D), A_x.dtype),
        scratch_shapes=[
            pltpu.VMEM((S // 2, D), u32),
            pltpu.VMEM((S // 2, D), u32),
            pltpu.VMEM((S, D), f32),
            pltpu.VMEM((D // 2, 3 * D), u32),
            pltpu.VMEM((D // 2, D), u32),
            pltpu.VMEM((D // 2, F), u32),
            pltpu.VMEM((D // 2, F), u32),
            pltpu.VMEM((F // 2, D), u32),
            pltpu.VMEM((4, 8, _HALO + _BM, 128), f32),
            pltpu.SemaphoreType.DMA((NB,)),
            pltpu.SemaphoreType.DMA((8,)),
        ],
        compiler_params=pltpu.CompilerParams(
            dimension_semantics=("arbitrary",),
            flags={"XLA_TPU_EVENLY_DISTRIBUTE_CRITICAL_NODES": True},
            vmem_limit_bytes=100 * 1024 * 1024,
        ),
    )(x, A_wqkv, A_wo, B_w1, B_w3, B_w2)
    return out.reshape(B, S0, D)
```

```python
import functools
import math

import jax
import jax.numpy as jnp
import jax.experimental.pallas as pl
import jax.experimental.pallas.tpu as pltpu

_H = 32
_W = 8
_DIL = 2
_HALO = 16
_BM = 256
_RG = 16
_F0 = 640
_FC = 512
_NEG = -1e9
_NA = 4
_TREE = 0
_GATE_W = 34
_GATE_J = 68
_GATE_S = 0
_JOUTER = 0
_NORMLATE = 1
_PACKO = 0
_PORDER = "qkv"


def _silu(x):
    return x * pl.reciprocal(1.0 + jnp.exp(-x), approx=True)


def _lane_exchange(blocks, lane):
    blocks = list(blocks)
    for b in range(3):
        sh = 2 << b
        m = (lane & sh) != 0
        for i in range(8):
            if i & (1 << b):
                continue
            lo, hi = blocks[i], blocks[i | (1 << b)]
            blocks[i] = jnp.where(m, pltpu.roll(hi, sh, 1), lo)
            blocks[i | (1 << b)] = jnp.where(m, hi, pltpu.roll(lo, 128 - sh, 1))
    return blocks


def _tree(fn, xs):
    xs = list(xs)
    while len(xs) > 1:
        xs = [fn(a, b) for a, b in zip(xs[0::2], xs[1::2])] + xs[len(xs) & ~1:]
    return xs[0]


def _xor_add(x, lane, sh):
    m = (lane & sh) != 0
    return x + jnp.where(m, pltpu.roll(x, sh, 1), pltpu.roll(x, 128 - sh, 1))


def _kernel(x_hbm, wqkv_hbm, wo_hbm, w1_hbm, w3_hbm, w2_hbm, o_ref,
            x_s, xn_s, acc_s, wqkv_s, wo_s, w1_s, w3_s, w2_s, att_s, sem_x, sem_w,
            *, S, D, F):
    NB = S // _BM
    step = pl.program_id(0)
    f32, bf16 = jnp.float32, jnp.bfloat16

    def b16(ref):
        return ref.bitcast(bf16)

    def ld(ref, rows, cols=slice(None)):
        st = rows.start // 2 if isinstance(rows.start, int) else pl.multiple_of(rows.start // 2, 8)
        return pltpu.bitcast(ref[pl.ds(st, rows.size // 2), cols], bf16)

    def x_copy(r):
        rows = pl.ds(r * _BM, _BM)
        return pltpu.make_async_copy(x_hbm.at[rows, :], b16(x_s).at[rows, :], sem_x.at[r])

    def w_copies_first():
        c = pl.ds(0, _F0)
        return [
            pltpu.make_async_copy(w1_hbm.at[:, c], b16(w1_s).at[:, c], sem_w.at[0]),
            pltpu.make_async_copy(w3_hbm.at[:, c], b16(w3_s).at[:, c], sem_w.at[1]),
            pltpu.make_async_copy(w2_hbm.at[c, :], b16(w2_s).at[c, :], sem_w.at[2]),
        ]

    def w_copies_rest():
        c = pl.ds(_F0, F - _F0)
        return [
            pltpu.make_async_copy(wqkv_hbm, b16(wqkv_s), sem_w.at[3]),
            pltpu.make_async_copy(w1_hbm.at[:, c], b16(w1_s).at[:, c], sem_w.at[4]),
            pltpu.make_async_copy(w3_hbm.at[:, c], b16(w3_s).at[:, c], sem_w.at[5]),
            pltpu.make_async_copy(w2_hbm.at[c, :], b16(w2_s).at[c, :], sem_w.at[6]),
            pltpu.make_async_copy(wo_hbm, b16(wo_s), sem_w.at[7]),
        ]

    def layernorm(r):
        rows = pl.ds(pl.multiple_of(r * _BM, _BM), _BM)
        x = ld(x_s, rows).astype(f32)
        mean = jnp.mean(x, axis=-1, keepdims=True)
        xc = x - mean
        var = jnp.mean(xc * xc, axis=-1, keepdims=True)
        xn = (xc * jax.lax.rsqrt(var + 1e-5)).astype(bf16)
        xn_s[pl.ds(pl.multiple_of(r * (_BM // 2), 8), _BM // 2), :] = pltpu.bitcast(xn, jnp.uint32)

    def ffn_chunk(xn, c0, cn, before=(None, None, None)):
        cols = pl.ds(c0, cn)

        def wait(i):
            if before[i] is not None:
                before[i].wait()

        wait(0)
        g = jnp.dot(xn, ld(w1_s, pl.ds(0, D), cols), preferred_element_type=f32)
        wait(1)
        u = jnp.dot(xn, ld(w3_s, pl.ds(0, D), cols), preferred_element_type=f32)
        h = (_silu(g) * u).astype(bf16)
        wait(2)
        return jnp.dot(h, ld(w2_s, cols), preferred_element_type=f32)

    @pl.when(step == 0)
    def _():
        x_copy(0).start()
        for c in w_copies_first():
            c.start()
        for r in range(1, NB):
            x_copy(r).start()
        for c in w_copies_rest():
            c.start()
        att_s[pl.ds(0, 2), :, pl.ds(0, _HALO), :] = jnp.zeros((2, 8, _HALO, 128), f32)
        x_copy(0).wait()
        layernorm(0)
        rows = pl.ds(0, _BM)
        acc_s[rows, :] = ffn_chunk(ld(xn_s, rows), 0, _F0, w_copies_first())
        x_copy(1).wait()
        layernorm(1)

    @pl.when(jnp.logical_and(step > 0, step < NB))
    def _():
        nxt = jnp.minimum(step + 1, NB - 1)

        @pl.when(step + 1 < NB)
        def _():
            x_copy(nxt).wait()

        rows = pl.ds(pl.multiple_of(step * _BM, _BM), _BM)
        xn = ld(xn_s, rows)
        layernorm(nxt)
        acc_s[rows, :] = ffn_chunk(xn, 0, _F0)

    @pl.when(step >= NB)
    def _():
        blk = step - NB

        @pl.when(blk == 0)
        def _():
            for c in w_copies_rest():
                c.wait()

        rows = pl.ds(pl.multiple_of(blk * _BM, _BM), _BM)
        xn = ld(xn_s, rows)
        lane = jax.lax.broadcasted_iota(jnp.int32, (_RG, 128), 1)

        def proj(c0):
            return jnp.dot(xn, ld(wqkv_s, pl.ds(0, D), pl.ds(c0, D)), preferred_element_type=f32)

        def groups(y):
            for g in range(_BM // _RG):
                yg = y[g * _RG:(g + 1) * _RG, :]
                yield g, _lane_exchange(
                    [yg[:, j * 128:(j + 1) * 128] for j in range(8)], lane)

        scale = (D // _H) ** -0.5
        log2e = math.log2(math.e)

        K, V, Q, O = 0, 1, 2, 3
        for name in _PORDER:
            src, dst = {"k": (1, K), "v": (2, V), "q": (0, Q)}[name]
            y = proj(src * D)
            if dst == Q:
                y = y * (scale * log2e)
            for g, blocks in groups(y):
                for j in range(8):
                    att_s[dst, j, pl.ds(_HALO + g * _RG, _RG), :] = blocks[j]

        chunks = []
        c0 = _F0
        while c0 < F:
            cn = min(_FC, F - c0)
            chunks.append((c0, cn))
            c0 += cn

        acc = acc_s[rows, :]
        for c0, cn in chunks[:_NA]:
            acc = acc + ffn_chunk(xn, c0, cn)

        zero = pl.multiple_of(jnp.minimum(blk, 0), 8)

        def grow(g):
            return (jax.lax.broadcasted_iota(jnp.int32, (_RG, 128), 0)
                    + (blk * _BM + g * _RG))

        red = _tree if _TREE else functools.reduce

        def gate(bit, val):
            if bit:
                att_s[O, 0, pl.ds(zero + _BM, 8), :] = val[:8]

        def weights_of(g):
            r0 = _HALO + g * _RG
            masked = g * _RG < (_W - 1) * _DIL
            logits = [None] * _W

            def term(j, w, q):
                return q * att_s[K, j, pl.ds(r0 - _DIL * w, _RG), :]

            if _JOUTER:
                for j in range(8):
                    q = att_s[Q, j, pl.ds(r0, _RG), :]
                    for w in range(_W):
                        t = term(j, w, q)
                        logits[w] = t if j == 0 else logits[w] + t
            else:
                qs = [att_s[Q, j, pl.ds(r0, _RG), :] for j in range(8)]
                for w in range(_W):
                    logits[w] = functools.reduce(
                        jnp.add, [term(j, w, qs[j]) for j in range(8)])
                    gate(_GATE_W >> w & 1, logits[w])
            for w in range(_W):
                l = _xor_add(logits[w], lane, 16)
                l = _xor_add(l, lane, 1)
                if masked and w > 0:
                    l = jnp.where(grow(g) >= _DIL * w, l, _NEG * log2e)
                logits[w] = l
            m = red(jnp.maximum, logits)
            e = [jnp.exp2(l - m) for l in logits]
            inv = pl.reciprocal(red(jnp.add, e), approx=True)
            gate(_GATE_S, inv)
            if _NORMLATE:
                return e, inv
            return [ei * inv for ei in e], None

        def mix_v(g, p, inv):
            r0 = _HALO + g * _RG
            masked = g * _RG < (_W - 1) * _DIL
            ob = []
            for j in range(8):
                if masked:
                    v0 = jnp.broadcast_to(att_s[V, j, pl.ds(_HALO, 1), :], (_RG, 128))
                oj = None
                for w in range(_W):
                    vw = att_s[V, j, pl.ds(r0 - _DIL * w, _RG), :]
                    if masked and w > 0:
                        vw = jnp.where(grow(g) >= _DIL * w, vw, v0)
                    t = p[w] * vw
                    oj = t if oj is None else oj + t
                if inv is not None:
                    oj = oj * inv
                gate(_GATE_J >> j & 1, oj)
                if _PACKO:
                    oj = pltpu.bitcast(oj.astype(bf16), f32)
                ob.append(oj)
            if _PACKO:
                return _lane_exchange(ob, lane[:_RG // 2])
            return _lane_exchange(ob, lane)

        n_groups = _BM // _RG
        og = _RG // 2 if _PACKO else _RG
        for g in range(n_groups):
            ob = mix_v(g, *weights_of(g))
            for j in range(8):
                att_s[O, j, pl.ds(zero + g * og, og), :] = ob[j]

        o = jnp.concatenate(
            [att_s[O, j, pl.ds(0, n_groups * og), :] for j in range(8)], axis=1)
        o = pltpu.bitcast(o, bf16) if _PACKO else o.astype(bf16)

        for t in (K, V):
            att_s[t, :, pl.ds(0, _HALO), :] = att_s[t, :, pl.ds(_BM, _HALO), :]

        s = jnp.dot(o, ld(wo_s, pl.ds(0, D)), preferred_element_type=f32)

        for c0, cn in chunks[_NA:]:
            acc = acc + ffn_chunk(xn, c0, cn)

        o_ref[...] = (ld(x_s, rows).astype(f32) + s * _silu(acc)).astype(o_ref.dtype)


@jax.jit
def pallas_recurrent_scan__sliding_local_dilated__glu_gated_swiglu__prompt_kernel(
    A_x: jax.Array,
    A_wqkv: jax.Array,
    A_wo: jax.Array,
    B_x: jax.Array,
    B_w1: jax.Array,
    B_w3: jax.Array,
    B_w2: jax.Array,
):
    del B_x
    B, S0, D = A_x.shape
    F = B_w1.shape[1]
    S = B * S0
    assert B == 1 and D == 1024 and S % _BM == 0
    NB = S // _BM
    x = A_x.reshape(S, D)
    f32, u32 = jnp.float32, jnp.uint32
    any_spec = pl.BlockSpec(memory_space=pl.ANY)
    out = pl.pallas_call(
        functools.partial(_kernel, S=S, D=D, F=F),
        grid=(2 * NB,),
        in_specs=[any_spec] * 6,
        out_specs=pl.BlockSpec((_BM, D), lambda i: (jnp.maximum(i - NB, 0), 0)),
        out_shape=jax.ShapeDtypeStruct((S, D), A_x.dtype),
        scratch_shapes=[
            pltpu.VMEM((S // 2, D), u32),
            pltpu.VMEM((S // 2, D), u32),
            pltpu.VMEM((S, D), f32),
            pltpu.VMEM((D // 2, 3 * D), u32),
            pltpu.VMEM((D // 2, D), u32),
            pltpu.VMEM((D // 2, F), u32),
            pltpu.VMEM((D // 2, F), u32),
            pltpu.VMEM((F // 2, D), u32),
            pltpu.VMEM((4, 8, _HALO + _BM, 128), f32),
            pltpu.SemaphoreType.DMA((NB,)),
            pltpu.SemaphoreType.DMA((8,)),
        ],
        compiler_params=pltpu.CompilerParams(
            dimension_semantics=("arbitrary",),
            flags={"XLA_TPU_EVENLY_DISTRIBUTE_CRITICAL_NODES": True},
            vmem_limit_bytes=100 * 1024 * 1024,
        ),
    )(x, A_wqkv, A_wo, B_w1, B_w3, B_w2)
    return out.reshape(B, S0, D)
```

```python
import functools
import math

import jax
import jax.numpy as jnp
import jax.experimental.pallas as pl
import jax.experimental.pallas.tpu as pltpu

_H = 32
_W = 8
_DIL = 2
_HALO = 16
_BM = 256
_RG = 16
_F0 = 768
_FIRST = (256,256,256)
_X1POS = 8
_OP = 2
_FC = 512
_NEG = -1e9
_NA = 4
_TREE = 0
_GATE_W = 34
_GATE_J = 68
_GATE_S = 0
_JOUTER = 0
_NORMLATE = 1
_PACKO = 0
_PORDER = "qkv"


def _silu(x):
    return x * pl.reciprocal(1.0 + jnp.exp(-x), approx=True)


def _lane_exchange(blocks, lane):
    blocks = list(blocks)
    for b in range(3):
        sh = 2 << b
        m = (lane & sh) != 0
        for i in range(8):
            if i & (1 << b):
                continue
            lo, hi = blocks[i], blocks[i | (1 << b)]
            blocks[i] = jnp.where(m, pltpu.roll(hi, sh, 1), lo)
            blocks[i | (1 << b)] = jnp.where(m, hi, pltpu.roll(lo, 128 - sh, 1))
    return blocks


def _tree(fn, xs):
    xs = list(xs)
    while len(xs) > 1:
        xs = [fn(a, b) for a, b in zip(xs[0::2], xs[1::2])] + xs[len(xs) & ~1:]
    return xs[0]


def _xor_add(x, lane, sh):
    m = (lane & sh) != 0
    return x + jnp.where(m, pltpu.roll(x, sh, 1), pltpu.roll(x, 128 - sh, 1))


def _kernel(x_hbm, wqkv_hbm, wo_hbm, w1_hbm, w3_hbm, w2_hbm, o_hbm,
            x_s, xn_s, acc_s, wqkv_s, wo_s, w1_s, w3_s, w2_s, att_s, out_s, sem_x, sem_w, sem_f, sem_o,
            *, S, D, F):
    NB = S // _BM
    step = pl.program_id(0)
    f32, bf16 = jnp.float32, jnp.bfloat16

    def b16(ref):
        return ref.bitcast(bf16)

    def ld(ref, rows, cols=slice(None)):
        st = rows.start // 2 if isinstance(rows.start, int) else pl.multiple_of(rows.start // 2, 8)
        return pltpu.bitcast(ref[pl.ds(st, rows.size // 2), cols], bf16)

    def x_copy(r):
        rows = pl.ds(r * _BM, _BM)
        return pltpu.make_async_copy(x_hbm.at[rows, :], b16(x_s).at[rows, :], sem_x.at[r])

    first = [(sum(_FIRST[:i]), n) for i, n in enumerate(_FIRST)]
    assert sum(_FIRST) == _F0

    def w_copies_first(i):
        c = pl.ds(*first[i])
        return [
            pltpu.make_async_copy(w1_hbm.at[:, c], b16(w1_s).at[:, c], sem_f.at[3 * i]),
            pltpu.make_async_copy(w3_hbm.at[:, c], b16(w3_s).at[:, c], sem_f.at[3 * i + 1]),
            pltpu.make_async_copy(w2_hbm.at[c, :], b16(w2_s).at[c, :], sem_f.at[3 * i + 2]),
        ]

    def w_copies_rest():
        c = pl.ds(_F0, F - _F0)
        return [
            pltpu.make_async_copy(wqkv_hbm, b16(wqkv_s), sem_w.at[0]),
            pltpu.make_async_copy(w1_hbm.at[:, c], b16(w1_s).at[:, c], sem_w.at[1]),
            pltpu.make_async_copy(w3_hbm.at[:, c], b16(w3_s).at[:, c], sem_w.at[2]),
            pltpu.make_async_copy(w2_hbm.at[c, :], b16(w2_s).at[c, :], sem_w.at[3]),
            pltpu.make_async_copy(wo_hbm, b16(wo_s), sem_w.at[4]),
        ]

    def layernorm(r):
        rows = pl.ds(pl.multiple_of(r * _BM, _BM), _BM)
        x = ld(x_s, rows).astype(f32)
        mean = jnp.mean(x, axis=-1, keepdims=True)
        xc = x - mean
        var = jnp.mean(xc * xc, axis=-1, keepdims=True)
        xn = (xc * jax.lax.rsqrt(var + 1e-5)).astype(bf16)
        xn_s[pl.ds(pl.multiple_of(r * (_BM // 2), 8), _BM // 2), :] = pltpu.bitcast(xn, jnp.uint32)

    def ffn_chunk(xn, c0, cn, before=(None, None, None)):
        cols = pl.ds(c0, cn)

        def wait(i):
            if before[i] is not None:
                before[i].wait()

        wait(0)
        g = jnp.dot(xn, ld(w1_s, pl.ds(0, D), cols), preferred_element_type=f32)
        wait(1)
        u = jnp.dot(xn, ld(w3_s, pl.ds(0, D), cols), preferred_element_type=f32)
        h = (_silu(g) * u).astype(bf16)
        wait(2)
        return jnp.dot(h, ld(w2_s, cols), preferred_element_type=f32)

    @pl.when(step == 0)
    def _():
        wf = [c for i in range(len(first)) for c in w_copies_first(i)]
        x_copy(0).start()
        for c in wf[:_X1POS] + [x_copy(1)] + wf[_X1POS:]:
            c.start()
        for r in range(2, NB):
            x_copy(r).start()
        for c in w_copies_rest():
            c.start()
        att_s[pl.ds(0, 2), :, pl.ds(0, _HALO), :] = jnp.zeros((2, 8, _HALO, 128), f32)
        x_copy(0).wait()
        layernorm(0)
        rows = pl.ds(0, _BM)

        class Wait:
            def __init__(self, n):
                self.n = n

            def wait(self):
                wf[self.n].wait()
                if self.n == _X1POS:
                    x_copy(1).wait()
                    layernorm(1)

        for i, (c0, cn) in enumerate(first):
            d = ffn_chunk(ld(xn_s, rows), c0, cn, [Wait(3 * i + k) for k in range(3)])
            acc_s[rows, :] = d if i == 0 else acc_s[rows, :] + d

    @pl.when(jnp.logical_and(step > 0, step < NB))
    def _():
        nxt = jnp.minimum(step + 1, NB - 1)

        @pl.when(step + 1 < NB)
        def _():
            x_copy(nxt).wait()

        rows = pl.ds(pl.multiple_of(step * _BM, _BM), _BM)
        xn = ld(xn_s, rows)
        layernorm(nxt)
        acc_s[rows, :] = ffn_chunk(xn, 0, _F0)

    @pl.when(step >= NB)
    def _():
        blk = step - NB

        @pl.when(blk == 0)
        def _():
            for c in w_copies_rest():
                c.wait()

        slot = blk % 2
        cw = D // _OP

        def out_copies(b, sl):
            r = pl.ds(pl.multiple_of(b * _BM, _BM), _BM)
            return [pltpu.make_async_copy(
                b16(out_s.at[sl]).at[:, pl.ds(i * cw, cw)],
                o_hbm.at[r, pl.ds(i * cw, cw)], sem_o.at[sl, i]) for i in range(_OP)]

        @pl.when(blk >= 2)
        def _():
            for c in out_copies(blk - 2, slot):
                c.wait()

        rows = pl.ds(pl.multiple_of(blk * _BM, _BM), _BM)
        xn = ld(xn_s, rows)
        lane = jax.lax.broadcasted_iota(jnp.int32, (_RG, 128), 1)

        def proj(c0):
            return jnp.dot(xn, ld(wqkv_s, pl.ds(0, D), pl.ds(c0, D)), preferred_element_type=f32)

        def groups(y):
            for g in range(_BM // _RG):
                yg = y[g * _RG:(g + 1) * _RG, :]
                yield g, _lane_exchange(
                    [yg[:, j * 128:(j + 1) * 128] for j in range(8)], lane)

        scale = (D // _H) ** -0.5
        log2e = math.log2(math.e)

        K, V, Q, O = 0, 1, 2, 3
        for name in _PORDER:
            src, dst = {"k": (1, K), "v": (2, V), "q": (0, Q)}[name]
            y = proj(src * D)
            if dst == Q:
                y = y * (scale * log2e)
            for g, blocks in groups(y):
                for j in range(8):
                    att_s[dst, j, pl.ds(_HALO + g * _RG, _RG), :] = blocks[j]

        chunks = []
        c0 = _F0
        while c0 < F:
            cn = min(_FC, F - c0)
            chunks.append((c0, cn))
            c0 += cn

        acc = acc_s[rows, :]
        for c0, cn in chunks[:_NA]:
            acc = acc + ffn_chunk(xn, c0, cn)

        zero = pl.multiple_of(jnp.minimum(blk, 0), 8)

        def grow(g):
            return (jax.lax.broadcasted_iota(jnp.int32, (_RG, 128), 0)
                    + (blk * _BM + g * _RG))

        red = _tree if _TREE else functools.reduce

        def gate(bit, val):
            if bit:
                att_s[O, 0, pl.ds(zero + _BM, 8), :] = val[:8]

        def weights_of(g):
            r0 = _HALO + g * _RG
            masked = g * _RG < (_W - 1) * _DIL
            logits = [None] * _W

            def term(j, w, q):
                return q * att_s[K, j, pl.ds(r0 - _DIL * w, _RG), :]

            if _JOUTER:
                for j in range(8):
                    q = att_s[Q, j, pl.ds(r0, _RG), :]
                    for w in range(_W):
                        t = term(j, w, q)
                        logits[w] = t if j == 0 else logits[w] + t
            else:
                qs = [att_s[Q, j, pl.ds(r0, _RG), :] for j in range(8)]
                for w in range(_W):
                    logits[w] = functools.reduce(
                        jnp.add, [term(j, w, qs[j]) for j in range(8)])
                    gate(_GATE_W >> w & 1, logits[w])
            for w in range(_W):
                l = _xor_add(logits[w], lane, 16)
                l = _xor_add(l, lane, 1)
                if masked and w > 0:
                    l = jnp.where(grow(g) >= _DIL * w, l, _NEG * log2e)
                logits[w] = l
            m = red(jnp.maximum, logits)
            e = [jnp.exp2(l - m) for l in logits]
            inv = pl.reciprocal(red(jnp.add, e), approx=True)
            gate(_GATE_S, inv)
            if _NORMLATE:
                return e, inv
            return [ei * inv for ei in e], None

        def mix_v(g, p, inv):
            r0 = _HALO + g * _RG
            masked = g * _RG < (_W - 1) * _DIL
            ob = []
            for j in range(8):
                if masked:
                    v0 = jnp.broadcast_to(att_s[V, j, pl.ds(_HALO, 1), :], (_RG, 128))
                oj = None
                for w in range(_W):
                    vw = att_s[V, j, pl.ds(r0 - _DIL * w, _RG), :]
                    if masked and w > 0:
                        vw = jnp.where(grow(g) >= _DIL * w, vw, v0)
                    t = p[w] * vw
                    oj = t if oj is None else oj + t
                if inv is not None:
                    oj = oj * inv
                gate(_GATE_J >> j & 1, oj)
                if _PACKO:
                    oj = pltpu.bitcast(oj.astype(bf16), f32)
                ob.append(oj)
            if _PACKO:
                return _lane_exchange(ob, lane[:_RG // 2])
            return _lane_exchange(ob, lane)

        n_groups = _BM // _RG
        og = _RG // 2 if _PACKO else _RG
        for g in range(n_groups):
            ob = mix_v(g, *weights_of(g))
            for j in range(8):
                att_s[O, j, pl.ds(zero + g * og, og), :] = ob[j]

        o = jnp.concatenate(
            [att_s[O, j, pl.ds(0, n_groups * og), :] for j in range(8)], axis=1)
        o = pltpu.bitcast(o, bf16) if _PACKO else o.astype(bf16)

        for t in (K, V):
            att_s[t, :, pl.ds(0, _HALO), :] = att_s[t, :, pl.ds(_BM, _HALO), :]

        s = jnp.dot(o, ld(wo_s, pl.ds(0, D)), preferred_element_type=f32)

        for c0, cn in chunks[_NA:]:
            acc = acc + ffn_chunk(xn, c0, cn)

        res = (ld(x_s, rows).astype(f32) + s * _silu(acc)).astype(bf16)
        res = pltpu.bitcast(res, jnp.uint32)
        for i, c in enumerate(out_copies(blk, slot)):
            cols = pl.ds(i * cw, cw)
            out_s[slot, :, cols] = res[:, i * cw:(i + 1) * cw]
            c.start()

        @pl.when(blk == NB - 1)
        def _():
            for c in out_copies(NB - 2, (NB - 2) % 2) + out_copies(NB - 1, (NB - 1) % 2):
                c.wait()


@jax.jit
def pallas_recurrent_scan__sliding_local_dilated__glu_gated_swiglu__prompt_kernel(
    A_x: jax.Array,
    A_wqkv: jax.Array,
    A_wo: jax.Array,
    B_x: jax.Array,
    B_w1: jax.Array,
    B_w3: jax.Array,
    B_w2: jax.Array,
):
    del B_x
    B, S0, D = A_x.shape
    F = B_w1.shape[1]
    S = B * S0
    assert B == 1 and D == 1024 and S % _BM == 0
    NB = S // _BM
    x = A_x.reshape(S, D)
    f32, u32 = jnp.float32, jnp.uint32
    any_spec = pl.BlockSpec(memory_space=pl.ANY)
    out = pl.pallas_call(
        functools.partial(_kernel, S=S, D=D, F=F),
        grid=(2 * NB,),
        in_specs=[any_spec] * 6,
        out_specs=any_spec,
        out_shape=jax.ShapeDtypeStruct((S, D), A_x.dtype),
        scratch_shapes=[
            pltpu.VMEM((S // 2, D), u32),
            pltpu.VMEM((S // 2, D), u32),
            pltpu.VMEM((S, D), f32),
            pltpu.VMEM((D // 2, 3 * D), u32),
            pltpu.VMEM((D // 2, D), u32),
            pltpu.VMEM((D // 2, F), u32),
            pltpu.VMEM((D // 2, F), u32),
            pltpu.VMEM((F // 2, D), u32),
            pltpu.VMEM((4, 8, _HALO + _BM, 128), f32),
            pltpu.VMEM((2, _BM // 2, D), u32),
            pltpu.SemaphoreType.DMA((NB,)),
            pltpu.SemaphoreType.DMA((5,)),
            pltpu.SemaphoreType.DMA((3 * len(_FIRST),)),
            pltpu.SemaphoreType.DMA((2, _OP)),
        ],
        compiler_params=pltpu.CompilerParams(
            dimension_semantics=("arbitrary",),
            flags={"XLA_TPU_EVENLY_DISTRIBUTE_CRITICAL_NODES": True},
            vmem_limit_bytes=100 * 1024 * 1024,
        ),
    )(x, A_wqkv, A_wo, B_w1, B_w3, B_w2)
    return out.reshape(B, S0, D)
```

```python
import functools
import math

import jax
import jax.numpy as jnp
import jax.experimental.pallas as pl
import jax.experimental.pallas.tpu as pltpu

_H = 32
_W = 8
_DIL = 2
_HALO = 16
_BM = 256
_RG = 16
_F0 = 768
_FIRST = (256,256,256)
_X1POS = 8
_OP = 2
_FC = 512
_NEG = -1e9
_NA = 4
_TREE = 0
_GATE_W = 34
_GATE_J = 68
_GATE_S = 0
_JOUTER = 0
_NORMLATE = 1
_PACKO = 0
_PORDER = "qkv"


def _silu(x):
    return x * pl.reciprocal(1.0 + jnp.exp(-x), approx=True)


def _lane_exchange(blocks, lane):
    blocks = list(blocks)
    for b in range(3):
        sh = 2 << b
        m = (lane & sh) != 0
        for i in range(8):
            if i & (1 << b):
                continue
            lo, hi = blocks[i], blocks[i | (1 << b)]
            blocks[i] = jnp.where(m, pltpu.roll(hi, sh, 1), lo)
            blocks[i | (1 << b)] = jnp.where(m, hi, pltpu.roll(lo, 128 - sh, 1))
    return blocks


def _tree(fn, xs):
    xs = list(xs)
    while len(xs) > 1:
        xs = [fn(a, b) for a, b in zip(xs[0::2], xs[1::2])] + xs[len(xs) & ~1:]
    return xs[0]


def _xor_add(x, lane, sh):
    m = (lane & sh) != 0
    return x + jnp.where(m, pltpu.roll(x, sh, 1), pltpu.roll(x, 128 - sh, 1))


def _kernel(x_hbm, wqkv_hbm, wo_hbm, w1_hbm, w3_hbm, w2_hbm, o_hbm,
            x_s, xn_s, acc_s, wqkv_s, wo_s, w1_s, w3_s, w2_s, att_s, out_s, sem_x, sem_w, sem_f, sem_o,
            *, S, D, F):
    NB = S // _BM
    f32, bf16 = jnp.float32, jnp.bfloat16

    def b16(ref):
        return ref.bitcast(bf16)

    def ld(ref, rows, cols=slice(None)):
        st = rows.start // 2 if isinstance(rows.start, int) else pl.multiple_of(rows.start // 2, 8)
        return pltpu.bitcast(ref[pl.ds(st, rows.size // 2), cols], bf16)

    def x_copy(r):
        rows = pl.ds(r * _BM, _BM)
        return pltpu.make_async_copy(x_hbm.at[rows, :], b16(x_s).at[rows, :], sem_x.at[r])

    first = [(sum(_FIRST[:i]), n) for i, n in enumerate(_FIRST)]
    assert sum(_FIRST) == _F0

    def w_copies_first(i):
        c = pl.ds(*first[i])
        return [
            pltpu.make_async_copy(w1_hbm.at[:, c], b16(w1_s).at[:, c], sem_f.at[3 * i]),
            pltpu.make_async_copy(w3_hbm.at[:, c], b16(w3_s).at[:, c], sem_f.at[3 * i + 1]),
            pltpu.make_async_copy(w2_hbm.at[c, :], b16(w2_s).at[c, :], sem_f.at[3 * i + 2]),
        ]

    def w_copies_rest():
        c = pl.ds(_F0, F - _F0)
        return [
            pltpu.make_async_copy(wqkv_hbm, b16(wqkv_s), sem_w.at[0]),
            pltpu.make_async_copy(w1_hbm.at[:, c], b16(w1_s).at[:, c], sem_w.at[1]),
            pltpu.make_async_copy(w3_hbm.at[:, c], b16(w3_s).at[:, c], sem_w.at[2]),
            pltpu.make_async_copy(w2_hbm.at[c, :], b16(w2_s).at[c, :], sem_w.at[3]),
            pltpu.make_async_copy(wo_hbm, b16(wo_s), sem_w.at[4]),
        ]

    def layernorm(r):
        rows = pl.ds(pl.multiple_of(r * _BM, _BM), _BM)
        x = ld(x_s, rows).astype(f32)
        mean = jnp.mean(x, axis=-1, keepdims=True)
        xc = x - mean
        var = jnp.mean(xc * xc, axis=-1, keepdims=True)
        xn = (xc * jax.lax.rsqrt(var + 1e-5)).astype(bf16)
        xn_s[pl.ds(pl.multiple_of(r * (_BM // 2), 8), _BM // 2), :] = pltpu.bitcast(xn, jnp.uint32)

    def ffn_chunk(xn, c0, cn, before=(None, None, None)):
        cols = pl.ds(c0, cn)

        def wait(i):
            if before[i] is not None:
                before[i].wait()

        wait(0)
        g = jnp.dot(xn, ld(w1_s, pl.ds(0, D), cols), preferred_element_type=f32)
        wait(1)
        u = jnp.dot(xn, ld(w3_s, pl.ds(0, D), cols), preferred_element_type=f32)
        h = (_silu(g) * u).astype(bf16)
        wait(2)
        return jnp.dot(h, ld(w2_s, cols), preferred_element_type=f32)

    def prologue():
        wf = [c for i in range(len(first)) for c in w_copies_first(i)]
        x_copy(0).start()
        for c in wf[:_X1POS] + [x_copy(1)] + wf[_X1POS:]:
            c.start()
        for r in range(2, NB):
            x_copy(r).start()
        for c in w_copies_rest():
            c.start()
        att_s[pl.ds(0, 2), :, pl.ds(0, _HALO), :] = jnp.zeros((2, 8, _HALO, 128), f32)
        x_copy(0).wait()
        layernorm(0)
        rows = pl.ds(0, _BM)

        class Wait:
            def __init__(self, n):
                self.n = n

            def wait(self):
                wf[self.n].wait()
                if self.n == _X1POS:
                    x_copy(1).wait()
                    layernorm(1)

        for i, (c0, cn) in enumerate(first):
            d = ffn_chunk(ld(xn_s, rows), c0, cn, [Wait(3 * i + k) for k in range(3)])
            acc_s[rows, :] = d if i == 0 else acc_s[rows, :] + d

    prologue()

    @pl.loop(1, NB)
    def _(step):
        nxt = jnp.minimum(step + 1, NB - 1)

        @pl.when(step + 1 < NB)
        def _():
            x_copy(nxt).wait()

        rows = pl.ds(pl.multiple_of(step * _BM, _BM), _BM)
        xn = ld(xn_s, rows)
        layernorm(nxt)
        acc_s[rows, :] = ffn_chunk(xn, 0, _F0)

    for c in w_copies_rest():
        c.wait()

    def out_copies(b, sl):
        r = pl.ds(pl.multiple_of(b * _BM, _BM), _BM)
        cw = D // _OP
        return [pltpu.make_async_copy(
            b16(out_s.at[sl]).at[:, pl.ds(i * cw, cw)],
            o_hbm.at[r, pl.ds(i * cw, cw)], sem_o.at[sl, i]) for i in range(_OP)]

    @pl.loop(0, NB)
    def _(blk):
        slot = blk % 2
        cw = D // _OP

        @pl.when(blk >= 2)
        def _():
            for c in out_copies(blk - 2, slot):
                c.wait()

        rows = pl.ds(pl.multiple_of(blk * _BM, _BM), _BM)
        xn = ld(xn_s, rows)
        lane = jax.lax.broadcasted_iota(jnp.int32, (_RG, 128), 1)

        def proj(c0):
            return jnp.dot(xn, ld(wqkv_s, pl.ds(0, D), pl.ds(c0, D)), preferred_element_type=f32)

        def groups(y):
            for g in range(_BM // _RG):
                yg = y[g * _RG:(g + 1) * _RG, :]
                yield g, _lane_exchange(
                    [yg[:, j * 128:(j + 1) * 128] for j in range(8)], lane)

        scale = (D // _H) ** -0.5
        log2e = math.log2(math.e)

        K, V, Q, O = 0, 1, 2, 3
        for name in _PORDER:
            src, dst = {"k": (1, K), "v": (2, V), "q": (0, Q)}[name]
            y = proj(src * D)
            if dst == Q:
                y = y * (scale * log2e)
            for g, blocks in groups(y):
                for j in range(8):
                    att_s[dst, j, pl.ds(_HALO + g * _RG, _RG), :] = blocks[j]

        chunks = []
        c0 = _F0
        while c0 < F:
            cn = min(_FC, F - c0)
            chunks.append((c0, cn))
            c0 += cn

        acc = acc_s[rows, :]
        for c0, cn in chunks[:_NA]:
            acc = acc + ffn_chunk(xn, c0, cn)

        zero = pl.multiple_of(jnp.minimum(blk, 0), 8)

        def grow(g):
            return (jax.lax.broadcasted_iota(jnp.int32, (_RG, 128), 0)
                    + (blk * _BM + g * _RG))

        red = _tree if _TREE else functools.reduce

        def gate(bit, val):
            if bit:
                att_s[O, 0, pl.ds(zero + _BM, 8), :] = val[:8]

        def weights_of(g):
            r0 = _HALO + g * _RG
            masked = g * _RG < (_W - 1) * _DIL
            logits = [None] * _W

            def term(j, w, q):
                return q * att_s[K, j, pl.ds(r0 - _DIL * w, _RG), :]

            if _JOUTER:
                for j in range(8):
                    q = att_s[Q, j, pl.ds(r0, _RG), :]
                    for w in range(_W):
                        t = term(j, w, q)
                        logits[w] = t if j == 0 else logits[w] + t
            else:
                qs = [att_s[Q, j, pl.ds(r0, _RG), :] for j in range(8)]
                for w in range(_W):
                    logits[w] = functools.reduce(
                        jnp.add, [term(j, w, qs[j]) for j in range(8)])
                    gate(_GATE_W >> w & 1, logits[w])
            for w in range(_W):
                l = _xor_add(logits[w], lane, 16)
                l = _xor_add(l, lane, 1)
                if masked and w > 0:
                    l = jnp.where(grow(g) >= _DIL * w, l, _NEG * log2e)
                logits[w] = l
            m = red(jnp.maximum, logits)
            e = [jnp.exp2(l - m) for l in logits]
            inv = pl.reciprocal(red(jnp.add, e), approx=True)
            gate(_GATE_S, inv)
            if _NORMLATE:
                return e, inv
            return [ei * inv for ei in e], None

        def mix_v(g, p, inv):
            r0 = _HALO + g * _RG
            masked = g * _RG < (_W - 1) * _DIL
            ob = []
            for j in range(8):
                if masked:
                    v0 = jnp.broadcast_to(att_s[V, j, pl.ds(_HALO, 1), :], (_RG, 128))
                oj = None
                for w in range(_W):
                    vw = att_s[V, j, pl.ds(r0 - _DIL * w, _RG), :]
                    if masked and w > 0:
                        vw = jnp.where(grow(g) >= _DIL * w, vw, v0)
                    t = p[w] * vw
                    oj = t if oj is None else oj + t
                if inv is not None:
                    oj = oj * inv
                gate(_GATE_J >> j & 1, oj)
                if _PACKO:
                    oj = pltpu.bitcast(oj.astype(bf16), f32)
                ob.append(oj)
            if _PACKO:
                return _lane_exchange(ob, lane[:_RG // 2])
            return _lane_exchange(ob, lane)

        n_groups = _BM // _RG
        og = _RG // 2 if _PACKO else _RG
        for g in range(n_groups):
            ob = mix_v(g, *weights_of(g))
            for j in range(8):
                att_s[O, j, pl.ds(zero + g * og, og), :] = ob[j]

        o = jnp.concatenate(
            [att_s[O, j, pl.ds(0, n_groups * og), :] for j in range(8)], axis=1)
        o = pltpu.bitcast(o, bf16) if _PACKO else o.astype(bf16)

        for t in (K, V):
            att_s[t, :, pl.ds(0, _HALO), :] = att_s[t, :, pl.ds(_BM, _HALO), :]

        s = jnp.dot(o, ld(wo_s, pl.ds(0, D)), preferred_element_type=f32)

        for c0, cn in chunks[_NA:]:
            acc = acc + ffn_chunk(xn, c0, cn)

        res = (ld(x_s, rows).astype(f32) + s * _silu(acc)).astype(bf16)
        res = pltpu.bitcast(res, jnp.uint32)
        for i, c in enumerate(out_copies(blk, slot)):
            cols = pl.ds(i * cw, cw)
            out_s[slot, :, cols] = res[:, i * cw:(i + 1) * cw]
            c.start()

    for c in out_copies(NB - 2, (NB - 2) % 2) + out_copies(NB - 1, (NB - 1) % 2):
        c.wait()


@jax.jit
def pallas_recurrent_scan__sliding_local_dilated__glu_gated_swiglu__prompt_kernel(
    A_x: jax.Array,
    A_wqkv: jax.Array,
    A_wo: jax.Array,
    B_x: jax.Array,
    B_w1: jax.Array,
    B_w3: jax.Array,
    B_w2: jax.Array,
):
    del B_x
    B, S0, D = A_x.shape
    F = B_w1.shape[1]
    S = B * S0
    assert B == 1 and D == 1024 and S % _BM == 0
    NB = S // _BM
    x = A_x.reshape(S, D)
    f32, u32 = jnp.float32, jnp.uint32
    any_spec = pl.BlockSpec(memory_space=pl.ANY)
    out = pl.pallas_call(
        functools.partial(_kernel, S=S, D=D, F=F),
        in_specs=[any_spec] * 6,
        out_specs=any_spec,
        out_shape=jax.ShapeDtypeStruct((S, D), A_x.dtype),
        scratch_shapes=[
            pltpu.VMEM((S // 2, D), u32),
            pltpu.VMEM((S // 2, D), u32),
            pltpu.VMEM((S, D), f32),
            pltpu.VMEM((D // 2, 3 * D), u32),
            pltpu.VMEM((D // 2, D), u32),
            pltpu.VMEM((D // 2, F), u32),
            pltpu.VMEM((D // 2, F), u32),
            pltpu.VMEM((F // 2, D), u32),
            pltpu.VMEM((4, 8, _HALO + _BM, 128), f32),
            pltpu.VMEM((2, _BM // 2, D), u32),
            pltpu.SemaphoreType.DMA((NB,)),
            pltpu.SemaphoreType.DMA((5,)),
            pltpu.SemaphoreType.DMA((3 * len(_FIRST),)),
            pltpu.SemaphoreType.DMA((2, _OP)),
        ],
        compiler_params=pltpu.CompilerParams(
            flags={"XLA_TPU_EVENLY_DISTRIBUTE_CRITICAL_NODES": True},
            vmem_limit_bytes=100 * 1024 * 1024,
        ),
    )(x, A_wqkv, A_wo, B_w1, B_w3, B_w2)
    return out.reshape(B, S0, D)
```

```python
import functools
import math

import jax
import jax.numpy as jnp
import jax.experimental.pallas as pl
import jax.experimental.pallas.tpu as pltpu

_H = 32
_W = 8
_DIL = 2
_HALO = 16
_BM = 256
_RG = 16
_F0 = 768
_FIRST = (256,256,256)
_X1POS = 8
_OP = 4
_FC = 512
_NEG = -1e9
_NA = 4
_TREE = 0
_GATE_W = 34
_GATE_J = 68
_GATE_S = 0
_JOUTER = 0
_NORMLATE = 1
_PACKO = 0
_PORDER = "qkv"


def _silu(x):
    return x * pl.reciprocal(1.0 + jnp.exp(-x), approx=True)


def _lane_exchange(blocks, lane):
    blocks = list(blocks)
    for b in range(3):
        sh = 2 << b
        m = (lane & sh) != 0
        for i in range(8):
            if i & (1 << b):
                continue
            lo, hi = blocks[i], blocks[i | (1 << b)]
            blocks[i] = jnp.where(m, pltpu.roll(hi, sh, 1), lo)
            blocks[i | (1 << b)] = jnp.where(m, hi, pltpu.roll(lo, 128 - sh, 1))
    return blocks


def _tree(fn, xs):
    xs = list(xs)
    while len(xs) > 1:
        xs = [fn(a, b) for a, b in zip(xs[0::2], xs[1::2])] + xs[len(xs) & ~1:]
    return xs[0]


def _xor_add(x, lane, sh):
    m = (lane & sh) != 0
    return x + jnp.where(m, pltpu.roll(x, sh, 1), pltpu.roll(x, 128 - sh, 1))


def _kernel(x_hbm, wqkv_hbm, wo_hbm, w1_hbm, w3_hbm, w2_hbm, o_hbm,
            x_s, xn_s, acc_s, wqkv_s, wo_s, w1_s, w3_s, w2_s, att_s, out_s, sem_x, sem_w, sem_f, sem_o,
            *, S, D, F):
    NB = S // _BM
    f32, bf16 = jnp.float32, jnp.bfloat16

    def b16(ref):
        return ref.bitcast(bf16)

    def ld(ref, rows, cols=slice(None)):
        st = rows.start // 2 if isinstance(rows.start, int) else pl.multiple_of(rows.start // 2, 8)
        return pltpu.bitcast(ref[pl.ds(st, rows.size // 2), cols], bf16)

    def x_copy(r):
        rows = pl.ds(r * _BM, _BM)
        return pltpu.make_async_copy(x_hbm.at[rows, :], b16(x_s).at[rows, :], sem_x.at[r])

    first = [(sum(_FIRST[:i]), n) for i, n in enumerate(_FIRST)]
    assert sum(_FIRST) == _F0

    def w_copies_first(i):
        c = pl.ds(*first[i])
        return [
            pltpu.make_async_copy(w1_hbm.at[:, c], b16(w1_s).at[:, c], sem_f.at[3 * i]),
            pltpu.make_async_copy(w3_hbm.at[:, c], b16(w3_s).at[:, c], sem_f.at[3 * i + 1]),
            pltpu.make_async_copy(w2_hbm.at[c, :], b16(w2_s).at[c, :], sem_f.at[3 * i + 2]),
        ]

    def w_copies_rest():
        c = pl.ds(_F0, F - _F0)
        return [
            pltpu.make_async_copy(wqkv_hbm, b16(wqkv_s), sem_w.at[0]),
            pltpu.make_async_copy(w1_hbm.at[:, c], b16(w1_s).at[:, c], sem_w.at[1]),
            pltpu.make_async_copy(w3_hbm.at[:, c], b16(w3_s).at[:, c], sem_w.at[2]),
            pltpu.make_async_copy(w2_hbm.at[c, :], b16(w2_s).at[c, :], sem_w.at[3]),
            pltpu.make_async_copy(wo_hbm, b16(wo_s), sem_w.at[4]),
        ]

    def layernorm(r):
        rows = pl.ds(pl.multiple_of(r * _BM, _BM), _BM)
        x = ld(x_s, rows).astype(f32)
        mean = jnp.mean(x, axis=-1, keepdims=True)
        xc = x - mean
        var = jnp.mean(xc * xc, axis=-1, keepdims=True)
        xn = (xc * jax.lax.rsqrt(var + 1e-5)).astype(bf16)
        xn_s[pl.ds(pl.multiple_of(r * (_BM // 2), 8), _BM // 2), :] = pltpu.bitcast(xn, jnp.uint32)

    def ffn_chunk(xn, c0, cn, before=(None, None, None)):
        cols = pl.ds(c0, cn)

        def wait(i):
            if before[i] is not None:
                before[i].wait()

        wait(0)
        g = jnp.dot(xn, ld(w1_s, pl.ds(0, D), cols), preferred_element_type=f32)
        wait(1)
        u = jnp.dot(xn, ld(w3_s, pl.ds(0, D), cols), preferred_element_type=f32)
        h = (_silu(g) * u).astype(bf16)
        wait(2)
        return jnp.dot(h, ld(w2_s, cols), preferred_element_type=f32)

    def prologue():
        wf = [c for i in range(len(first)) for c in w_copies_first(i)]
        x_copy(0).start()
        for c in wf[:_X1POS] + [x_copy(1)] + wf[_X1POS:]:
            c.start()
        for r in range(2, NB):
            x_copy(r).start()
        for c in w_copies_rest():
            c.start()
        att_s[pl.ds(0, 2), :, pl.ds(0, _HALO), :] = jnp.zeros((2, 8, _HALO, 128), f32)
        x_copy(0).wait()
        layernorm(0)
        rows = pl.ds(0, _BM)

        class Wait:
            def __init__(self, n):
                self.n = n

            def wait(self):
                wf[self.n].wait()
                if self.n == _X1POS:
                    x_copy(1).wait()
                    layernorm(1)

        for i, (c0, cn) in enumerate(first):
            d = ffn_chunk(ld(xn_s, rows), c0, cn, [Wait(3 * i + k) for k in range(3)])
            acc_s[rows, :] = d if i == 0 else acc_s[rows, :] + d

    prologue()

    @pl.loop(1, NB)
    def _(step):
        nxt = jnp.minimum(step + 1, NB - 1)

        @pl.when(step + 1 < NB)
        def _():
            x_copy(nxt).wait()

        rows = pl.ds(pl.multiple_of(step * _BM, _BM), _BM)
        xn = ld(xn_s, rows)
        layernorm(nxt)
        acc_s[rows, :] = ffn_chunk(xn, 0, _F0)

    for c in w_copies_rest():
        c.wait()

    def out_copies(b, sl):
        r = pl.ds(pl.multiple_of(b * _BM, _BM), _BM)
        cw = D // _OP
        return [pltpu.make_async_copy(
            out_s.at[sl, :, pl.ds(i * cw, cw)],
            o_hbm.at[r, pl.ds(i * cw, cw)], sem_o.at[sl, i]) for i in range(_OP)]

    @pl.loop(0, NB)
    def _(blk):
        slot = blk % 2
        cw = D // _OP

        @pl.when(blk >= 2)
        def _():
            for c in out_copies(blk - 2, slot):
                c.wait()

        rows = pl.ds(pl.multiple_of(blk * _BM, _BM), _BM)
        xn = ld(xn_s, rows)
        lane = jax.lax.broadcasted_iota(jnp.int32, (_RG, 128), 1)

        def proj(c0):
            return jnp.dot(xn, ld(wqkv_s, pl.ds(0, D), pl.ds(c0, D)), preferred_element_type=f32)

        def groups(y):
            for g in range(_BM // _RG):
                yg = y[g * _RG:(g + 1) * _RG, :]
                yield g, _lane_exchange(
                    [yg[:, j * 128:(j + 1) * 128] for j in range(8)], lane)

        scale = (D // _H) ** -0.5
        log2e = math.log2(math.e)

        K, V, Q, O = 0, 1, 2, 3
        for name in _PORDER:
            src, dst = {"k": (1, K), "v": (2, V), "q": (0, Q)}[name]
            y = proj(src * D)
            if dst == Q:
                y = y * (scale * log2e)
            for g, blocks in groups(y):
                for j in range(8):
                    att_s[dst, j, pl.ds(_HALO + g * _RG, _RG), :] = blocks[j]

        chunks = []
        c0 = _F0
        while c0 < F:
            cn = min(_FC, F - c0)
            chunks.append((c0, cn))
            c0 += cn

        acc = acc_s[rows, :]
        for c0, cn in chunks[:_NA]:
            acc = acc + ffn_chunk(xn, c0, cn)

        zero = pl.multiple_of(jnp.minimum(blk, 0), 8)

        def grow(g):
            return (jax.lax.broadcasted_iota(jnp.int32, (_RG, 128), 0)
                    + (blk * _BM + g * _RG))

        red = _tree if _TREE else functools.reduce

        def gate(bit, val):
            if bit:
                att_s[O, 0, pl.ds(zero + _BM, 8), :] = val[:8]

        def weights_of(g):
            r0 = _HALO + g * _RG
            masked = g * _RG < (_W - 1) * _DIL
            logits = [None] * _W

            def term(j, w, q):
                return q * att_s[K, j, pl.ds(r0 - _DIL * w, _RG), :]

            if _JOUTER:
                for j in range(8):
                    q = att_s[Q, j, pl.ds(r0, _RG), :]
                    for w in range(_W):
                        t = term(j, w, q)
                        logits[w] = t if j == 0 else logits[w] + t
            else:
                qs = [att_s[Q, j, pl.ds(r0, _RG), :] for j in range(8)]
                for w in range(_W):
                    logits[w] = functools.reduce(
                        jnp.add, [term(j, w, qs[j]) for j in range(8)])
                    gate(_GATE_W >> w & 1, logits[w])
            for w in range(_W):
                l = _xor_add(logits[w], lane, 16)
                l = _xor_add(l, lane, 1)
                if masked and w > 0:
                    l = jnp.where(grow(g) >= _DIL * w, l, _NEG * log2e)
                logits[w] = l
            m = red(jnp.maximum, logits)
            e = [jnp.exp2(l - m) for l in logits]
            inv = pl.reciprocal(red(jnp.add, e), approx=True)
            gate(_GATE_S, inv)
            if _NORMLATE:
                return e, inv
            return [ei * inv for ei in e], None

        def mix_v(g, p, inv):
            r0 = _HALO + g * _RG
            masked = g * _RG < (_W - 1) * _DIL
            ob = []
            for j in range(8):
                if masked:
                    v0 = jnp.broadcast_to(att_s[V, j, pl.ds(_HALO, 1), :], (_RG, 128))
                oj = None
                for w in range(_W):
                    vw = att_s[V, j, pl.ds(r0 - _DIL * w, _RG), :]
                    if masked and w > 0:
                        vw = jnp.where(grow(g) >= _DIL * w, vw, v0)
                    t = p[w] * vw
                    oj = t if oj is None else oj + t
                if inv is not None:
                    oj = oj * inv
                gate(_GATE_J >> j & 1, oj)
                if _PACKO:
                    oj = pltpu.bitcast(oj.astype(bf16), f32)
                ob.append(oj)
            if _PACKO:
                return _lane_exchange(ob, lane[:_RG // 2])
            return _lane_exchange(ob, lane)

        n_groups = _BM // _RG
        og = _RG // 2 if _PACKO else _RG
        for g in range(n_groups):
            ob = mix_v(g, *weights_of(g))
            for j in range(8):
                att_s[O, j, pl.ds(zero + g * og, og), :] = ob[j]

        o = jnp.concatenate(
            [att_s[O, j, pl.ds(0, n_groups * og), :] for j in range(8)], axis=1)
        o = pltpu.bitcast(o, bf16) if _PACKO else o.astype(bf16)

        for t in (K, V):
            att_s[t, :, pl.ds(0, _HALO), :] = att_s[t, :, pl.ds(_BM, _HALO), :]

        s = jnp.dot(o, ld(wo_s, pl.ds(0, D)), preferred_element_type=f32)

        for c0, cn in chunks[_NA:]:
            acc = acc + ffn_chunk(xn, c0, cn)

        res = (ld(x_s, rows).astype(f32) + s * _silu(acc)).astype(bf16)
        for i, c in enumerate(out_copies(blk, slot)):
            cols = pl.ds(i * cw, cw)
            out_s[slot, :, cols] = res[:, i * cw:(i + 1) * cw]
            c.start()

    for c in out_copies(NB - 2, (NB - 2) % 2) + out_copies(NB - 1, (NB - 1) % 2):
        c.wait()


@jax.jit
def pallas_recurrent_scan__sliding_local_dilated__glu_gated_swiglu__prompt_kernel(
    A_x: jax.Array,
    A_wqkv: jax.Array,
    A_wo: jax.Array,
    B_x: jax.Array,
    B_w1: jax.Array,
    B_w3: jax.Array,
    B_w2: jax.Array,
):
    del B_x
    B, S0, D = A_x.shape
    F = B_w1.shape[1]
    S = B * S0
    assert B == 1 and D == 1024 and S % _BM == 0
    NB = S // _BM
    x = A_x.reshape(S, D)
    f32, u32, bf16 = jnp.float32, jnp.uint32, jnp.bfloat16
    any_spec = pl.BlockSpec(memory_space=pl.ANY)
    out = pl.pallas_call(
        functools.partial(_kernel, S=S, D=D, F=F),
        in_specs=[any_spec] * 6,
        out_specs=any_spec,
        out_shape=jax.ShapeDtypeStruct((S, D), A_x.dtype),
        scratch_shapes=[
            pltpu.VMEM((S // 2, D), u32),
            pltpu.VMEM((S // 2, D), u32),
            pltpu.VMEM((S, D), f32),
            pltpu.VMEM((D // 2, 3 * D), u32),
            pltpu.VMEM((D // 2, D), u32),
            pltpu.VMEM((D // 2, F), u32),
            pltpu.VMEM((D // 2, F), u32),
            pltpu.VMEM((F // 2, D), u32),
            pltpu.VMEM((4, 8, _HALO + _BM, 128), f32),
            pltpu.VMEM((2, _BM, D), bf16),
            pltpu.SemaphoreType.DMA((NB,)),
            pltpu.SemaphoreType.DMA((5,)),
            pltpu.SemaphoreType.DMA((3 * len(_FIRST),)),
            pltpu.SemaphoreType.DMA((2, _OP)),
        ],
        compiler_params=pltpu.CompilerParams(
            flags={"XLA_TPU_EVENLY_DISTRIBUTE_CRITICAL_NODES": True},
            vmem_limit_bytes=100 * 1024 * 1024,
        ),
    )(x, A_wqkv, A_wo, B_w1, B_w3, B_w2)
    return out.reshape(B, S0, D)
```

```python
import functools
import math

import jax
import jax.numpy as jnp
import jax.experimental.pallas as pl
import jax.experimental.pallas.tpu as pltpu

_H = 32
_W = 8
_DIL = 2
_HALO = 16
_BM = 256
_RG = 16
_F0 = 896
_FIRST = (256,256,384)
_X1POS = 8
_OP = 4
_PACKED = 1
_FC = 896
_NEG = -1e9
_NA = 3
_TREE = 0
_GATE_W = 34
_GATE_J = 34
_GATE_S = 0
_JOUTER = 0
_NORMLATE = 1
_PACKO = 0
_PORDER = "kvq"


def _silu(x):
    return x * pl.reciprocal(1.0 + jnp.exp(-x), approx=True)


def _lane_exchange(blocks, lane):
    blocks = list(blocks)
    for b in range(3):
        sh = 2 << b
        m = (lane & sh) != 0
        for i in range(8):
            if i & (1 << b):
                continue
            lo, hi = blocks[i], blocks[i | (1 << b)]
            blocks[i] = jnp.where(m, pltpu.roll(hi, sh, 1), lo)
            blocks[i | (1 << b)] = jnp.where(m, hi, pltpu.roll(lo, 128 - sh, 1))
    return blocks


def _tree(fn, xs):
    xs = list(xs)
    while len(xs) > 1:
        xs = [fn(a, b) for a, b in zip(xs[0::2], xs[1::2])] + xs[len(xs) & ~1:]
    return xs[0]


def _xor_add(x, lane, sh):
    m = (lane & sh) != 0
    return x + jnp.where(m, pltpu.roll(x, sh, 1), pltpu.roll(x, 128 - sh, 1))


def _kernel(x_hbm, wqkv_hbm, wo_hbm, w1_hbm, w3_hbm, w2_hbm, o_hbm,
            x_s, xn_s, acc_s, wqkv_s, wo_s, w1_s, w3_s, w2_s, att_s, out_s, sem_x, sem_w, sem_f, sem_o,
            *, S, D, F):
    NB = S // _BM
    f32, bf16 = jnp.float32, jnp.bfloat16

    def b16(ref):
        return ref.bitcast(bf16) if _PACKED else ref

    def ld(ref, rows, cols=slice(None)):
        if not _PACKED:
            return ref[rows, cols]
        st = rows.start // 2 if isinstance(rows.start, int) else pl.multiple_of(rows.start // 2, 8)
        return pltpu.bitcast(ref[pl.ds(st, rows.size // 2), cols], bf16)

    def x_copy(r):
        rows = pl.ds(r * _BM, _BM)
        return pltpu.make_async_copy(x_hbm.at[rows, :], b16(x_s).at[rows, :], sem_x.at[r])

    first = [(sum(_FIRST[:i]), n) for i, n in enumerate(_FIRST)]
    assert sum(_FIRST) == _F0

    def w_copies_first(i):
        c = pl.ds(*first[i])
        return [
            pltpu.make_async_copy(w1_hbm.at[:, c], b16(w1_s).at[:, c], sem_f.at[3 * i]),
            pltpu.make_async_copy(w3_hbm.at[:, c], b16(w3_s).at[:, c], sem_f.at[3 * i + 1]),
            pltpu.make_async_copy(w2_hbm.at[c, :], b16(w2_s).at[c, :], sem_f.at[3 * i + 2]),
        ]

    def w_copies_rest():
        c = pl.ds(_F0, F - _F0)
        return [
            pltpu.make_async_copy(wqkv_hbm, b16(wqkv_s), sem_w.at[0]),
            pltpu.make_async_copy(w1_hbm.at[:, c], b16(w1_s).at[:, c], sem_w.at[1]),
            pltpu.make_async_copy(w3_hbm.at[:, c], b16(w3_s).at[:, c], sem_w.at[2]),
            pltpu.make_async_copy(w2_hbm.at[c, :], b16(w2_s).at[c, :], sem_w.at[3]),
            pltpu.make_async_copy(wo_hbm, b16(wo_s), sem_w.at[4]),
        ]

    def layernorm(r):
        rows = pl.ds(pl.multiple_of(r * _BM, _BM), _BM)
        x = ld(x_s, rows).astype(f32)
        mean = jnp.mean(x, axis=-1, keepdims=True)
        xc = x - mean
        var = jnp.mean(xc * xc, axis=-1, keepdims=True)
        xn = (xc * jax.lax.rsqrt(var + 1e-5)).astype(bf16)
        if _PACKED:
            xn_s[pl.ds(pl.multiple_of(r * (_BM // 2), 8), _BM // 2), :] = pltpu.bitcast(xn, jnp.uint32)
        else:
            xn_s[rows, :] = xn

    def ffn_chunk(xn, c0, cn, before=(None, None, None)):
        cols = pl.ds(c0, cn)

        def wait(i):
            if before[i] is not None:
                before[i].wait()

        wait(0)
        g = jnp.dot(xn, ld(w1_s, pl.ds(0, D), cols), preferred_element_type=f32)
        wait(1)
        u = jnp.dot(xn, ld(w3_s, pl.ds(0, D), cols), preferred_element_type=f32)
        h = (_silu(g) * u).astype(bf16)
        wait(2)
        return jnp.dot(h, ld(w2_s, cols), preferred_element_type=f32)

    def prologue():
        wf = [c for i in range(len(first)) for c in w_copies_first(i)]
        x_copy(0).start()
        for c in wf[:_X1POS] + [x_copy(1)] + wf[_X1POS:]:
            c.start()
        for r in range(2, NB):
            x_copy(r).start()
        for c in w_copies_rest():
            c.start()
        att_s[pl.ds(0, 2), :, pl.ds(0, _HALO), :] = jnp.zeros((2, 8, _HALO, 128), f32)
        x_copy(0).wait()
        layernorm(0)
        rows = pl.ds(0, _BM)

        class Wait:
            def __init__(self, n):
                self.n = n

            def wait(self):
                wf[self.n].wait()
                if self.n == _X1POS:
                    x_copy(1).wait()
                    layernorm(1)

        for i, (c0, cn) in enumerate(first):
            d = ffn_chunk(ld(xn_s, rows), c0, cn, [Wait(3 * i + k) for k in range(3)])
            acc_s[rows, :] = d if i == 0 else acc_s[rows, :] + d

    prologue()

    @pl.loop(1, NB)
    def _(step):
        nxt = jnp.minimum(step + 1, NB - 1)

        @pl.when(step + 1 < NB)
        def _():
            x_copy(nxt).wait()

        rows = pl.ds(pl.multiple_of(step * _BM, _BM), _BM)
        xn = ld(xn_s, rows)
        layernorm(nxt)
        acc_s[rows, :] = ffn_chunk(xn, 0, _F0)

    for c in w_copies_rest():
        c.wait()

    def out_copies(b, sl):
        r = pl.ds(pl.multiple_of(b * _BM, _BM), _BM)
        cw = D // _OP
        return [pltpu.make_async_copy(
            out_s.at[sl, :, pl.ds(i * cw, cw)],
            o_hbm.at[r, pl.ds(i * cw, cw)], sem_o.at[sl, i]) for i in range(_OP)]

    @pl.loop(0, NB)
    def _(blk):
        slot = blk % 2
        cw = D // _OP

        @pl.when(blk >= 2)
        def _():
            for c in out_copies(blk - 2, slot):
                c.wait()

        rows = pl.ds(pl.multiple_of(blk * _BM, _BM), _BM)
        xn = ld(xn_s, rows)
        lane = jax.lax.broadcasted_iota(jnp.int32, (_RG, 128), 1)

        def proj(c0):
            return jnp.dot(xn, ld(wqkv_s, pl.ds(0, D), pl.ds(c0, D)), preferred_element_type=f32)

        def groups(y):
            for g in range(_BM // _RG):
                yg = y[g * _RG:(g + 1) * _RG, :]
                yield g, _lane_exchange(
                    [yg[:, j * 128:(j + 1) * 128] for j in range(8)], lane)

        scale = (D // _H) ** -0.5
        log2e = math.log2(math.e)

        K, V, Q, O = 0, 1, 2, 3
        for name in _PORDER:
            src, dst = {"k": (1, K), "v": (2, V), "q": (0, Q)}[name]
            y = proj(src * D)
            if dst == Q:
                y = y * (scale * log2e)
            for g, blocks in groups(y):
                for j in range(8):
                    att_s[dst, j, pl.ds(_HALO + g * _RG, _RG), :] = blocks[j]

        chunks = []
        c0 = _F0
        while c0 < F:
            cn = min(_FC, F - c0)
            chunks.append((c0, cn))
            c0 += cn

        acc = acc_s[rows, :]
        for c0, cn in chunks[:_NA]:
            acc = acc + ffn_chunk(xn, c0, cn)

        zero = pl.multiple_of(jnp.minimum(blk, 0), 8)

        def grow(g):
            return (jax.lax.broadcasted_iota(jnp.int32, (_RG, 128), 0)
                    + (blk * _BM + g * _RG))

        red = _tree if _TREE else functools.reduce

        def gate(bit, val):
            if bit:
                att_s[O, 0, pl.ds(zero + _BM, 8), :] = val[:8]

        def weights_of(g):
            r0 = _HALO + g * _RG
            masked = g * _RG < (_W - 1) * _DIL
            logits = [None] * _W

            def term(j, w, q):
                return q * att_s[K, j, pl.ds(r0 - _DIL * w, _RG), :]

            if _JOUTER:
                for j in range(8):
                    q = att_s[Q, j, pl.ds(r0, _RG), :]
                    for w in range(_W):
                        t = term(j, w, q)
                        logits[w] = t if j == 0 else logits[w] + t
            else:
                qs = [att_s[Q, j, pl.ds(r0, _RG), :] for j in range(8)]
                for w in range(_W):
                    logits[w] = functools.reduce(
                        jnp.add, [term(j, w, qs[j]) for j in range(8)])
                    gate(_GATE_W >> w & 1, logits[w])
            for w in range(_W):
                l = _xor_add(logits[w], lane, 16)
                l = _xor_add(l, lane, 1)
                if masked and w > 0:
                    l = jnp.where(grow(g) >= _DIL * w, l, _NEG * log2e)
                logits[w] = l
            m = red(jnp.maximum, logits)
            e = [jnp.exp2(l - m) for l in logits]
            inv = pl.reciprocal(red(jnp.add, e), approx=True)
            gate(_GATE_S, inv)
            if _NORMLATE:
                return e, inv
            return [ei * inv for ei in e], None

        def mix_v(g, p, inv):
            r0 = _HALO + g * _RG
            masked = g * _RG < (_W - 1) * _DIL
            ob = []
            for j in range(8):
                if masked:
                    v0 = jnp.broadcast_to(att_s[V, j, pl.ds(_HALO, 1), :], (_RG, 128))
                oj = None
                for w in range(_W):
                    vw = att_s[V, j, pl.ds(r0 - _DIL * w, _RG), :]
                    if masked and w > 0:
                        vw = jnp.where(grow(g) >= _DIL * w, vw, v0)
                    t = p[w] * vw
                    oj = t if oj is None else oj + t
                if inv is not None:
                    oj = oj * inv
                gate(_GATE_J >> j & 1, oj)
                if _PACKO:
                    oj = pltpu.bitcast(oj.astype(bf16), f32)
                ob.append(oj)
            if _PACKO:
                return _lane_exchange(ob, lane[:_RG // 2])
            return _lane_exchange(ob, lane)

        n_groups = _BM // _RG
        og = _RG // 2 if _PACKO else _RG
        for g in range(n_groups):
            ob = mix_v(g, *weights_of(g))
            for j in range(8):
                att_s[O, j, pl.ds(zero + g * og, og), :] = ob[j]

        o = jnp.concatenate(
            [att_s[O, j, pl.ds(0, n_groups * og), :] for j in range(8)], axis=1)
        o = pltpu.bitcast(o, bf16) if _PACKO else o.astype(bf16)

        for t in (K, V):
            att_s[t, :, pl.ds(0, _HALO), :] = att_s[t, :, pl.ds(_BM, _HALO), :]

        s = jnp.dot(o, ld(wo_s, pl.ds(0, D)), preferred_element_type=f32)

        for c0, cn in chunks[_NA:]:
            acc = acc + ffn_chunk(xn, c0, cn)

        res = (ld(x_s, rows).astype(f32) + s * _silu(acc)).astype(bf16)
        for i, c in enumerate(out_copies(blk, slot)):
            cols = pl.ds(i * cw, cw)
            out_s[slot, :, cols] = res[:, i * cw:(i + 1) * cw]
            c.start()

    for c in out_copies(NB - 2, (NB - 2) % 2) + out_copies(NB - 1, (NB - 1) % 2):
        c.wait()


@jax.jit
def pallas_recurrent_scan__sliding_local_dilated__glu_gated_swiglu__prompt_kernel(
    A_x: jax.Array,
    A_wqkv: jax.Array,
    A_wo: jax.Array,
    B_x: jax.Array,
    B_w1: jax.Array,
    B_w3: jax.Array,
    B_w2: jax.Array,
):
    del B_x
    B, S0, D = A_x.shape
    F = B_w1.shape[1]
    S = B * S0
    assert B == 1 and D == 1024 and S % _BM == 0
    NB = S // _BM
    x = A_x.reshape(S, D)
    f32, u32, bf16 = jnp.float32, jnp.uint32, jnp.bfloat16
    if _PACKED:
        w16 = lambda r, c: pltpu.VMEM((r // 2, c), u32)
    else:
        w16 = lambda r, c: pltpu.VMEM((r, c), bf16)
    any_spec = pl.BlockSpec(memory_space=pl.ANY)
    out = pl.pallas_call(
        functools.partial(_kernel, S=S, D=D, F=F),
        in_specs=[any_spec] * 6,
        out_specs=any_spec,
        out_shape=jax.ShapeDtypeStruct((S, D), A_x.dtype),
        scratch_shapes=[
            w16(S, D),
            w16(S, D),
            pltpu.VMEM((S, D), f32),
            w16(D, 3 * D),
            w16(D, D),
            w16(D, F),
            w16(D, F),
            w16(F, D),
            pltpu.VMEM((4, 8, _HALO + _BM, 128), f32),
            pltpu.VMEM((2, _BM, D), bf16),
            pltpu.SemaphoreType.DMA((NB,)),
            pltpu.SemaphoreType.DMA((5,)),
            pltpu.SemaphoreType.DMA((3 * len(_FIRST),)),
            pltpu.SemaphoreType.DMA((2, _OP)),
        ],
        compiler_params=pltpu.CompilerParams(
            flags={"XLA_TPU_EVENLY_DISTRIBUTE_CRITICAL_NODES": True},
            vmem_limit_bytes=100 * 1024 * 1024,
        ),
    )(x, A_wqkv, A_wo, B_w1, B_w3, B_w2)
    return out.reshape(B, S0, D)
```

```python
import functools
import math

import jax
import jax.numpy as jnp
import jax.experimental.pallas as pl
import jax.experimental.pallas.tpu as pltpu

_H = 32
_W = 8
_DIL = 2
_NEG = -1e9
_HALO = 16
_BM = 256
_RG = 16
_F0 = 896
_FIRST = (256, 256, 384)
_FC = 896
_OP = 4
_GATE_W = (1, 5)
_GATE_J = (1, 5)

_F32, _BF16, _U32 = jnp.float32, jnp.bfloat16, jnp.uint32


def _silu(x):
    return x * pl.reciprocal(1.0 + jnp.exp(-x), approx=True)


def _lane_exchange(blocks, lane):
    blocks = list(blocks)
    for b in range(3):
        sh = 2 << b
        m = (lane & sh) != 0
        for i in range(8):
            if i & (1 << b):
                continue
            lo, hi = blocks[i], blocks[i | (1 << b)]
            blocks[i] = jnp.where(m, pltpu.roll(hi, sh, 1), lo)
            blocks[i | (1 << b)] = jnp.where(m, hi, pltpu.roll(lo, 128 - sh, 1))
    return blocks


def _xor_add(x, lane, sh):
    m = (lane & sh) != 0
    return x + jnp.where(m, pltpu.roll(x, sh, 1), pltpu.roll(x, 128 - sh, 1))


def _kernel(x_hbm, wqkv_hbm, wo_hbm, w1_hbm, w3_hbm, w2_hbm, o_hbm,
            x_s, xn_s, acc_s, wqkv_s, wo_s, w1_s, w3_s, w2_s, att_s, out_s,
            sem_x, sem_w, sem_f, sem_o, *, S, D, F):
    NB = S // _BM

    def b16(ref):
        return ref.bitcast(_BF16)

    def ld(ref, rows, cols=slice(None)):
        if isinstance(rows.start, int):
            start = rows.start // 2
        else:
            start = pl.multiple_of(rows.start // 2, 8)
        return pltpu.bitcast(ref[pl.ds(start, rows.size // 2), cols], _BF16)

    def x_copy(r):
        rows = pl.ds(r * _BM, _BM)
        return pltpu.make_async_copy(x_hbm.at[rows, :], b16(x_s).at[rows, :], sem_x.at[r])

    def ffn_copies(cols, sem, i):
        return [
            pltpu.make_async_copy(w1_hbm.at[:, cols], b16(w1_s).at[:, cols], sem.at[i]),
            pltpu.make_async_copy(w3_hbm.at[:, cols], b16(w3_s).at[:, cols], sem.at[i + 1]),
            pltpu.make_async_copy(w2_hbm.at[cols, :], b16(w2_s).at[cols, :], sem.at[i + 2]),
        ]

    first = [(sum(_FIRST[:i]), n) for i, n in enumerate(_FIRST)]
    assert sum(_FIRST) == _F0 and (F - _F0) % _FC == 0

    def w_copies_rest():
        return ([pltpu.make_async_copy(wqkv_hbm, b16(wqkv_s), sem_w.at[0])]
                + ffn_copies(pl.ds(_F0, F - _F0), sem_w, 1)
                + [pltpu.make_async_copy(wo_hbm, b16(wo_s), sem_w.at[4])])

    def out_copies(blk, slot):
        rows = pl.ds(pl.multiple_of(blk * _BM, _BM), _BM)
        cw = D // _OP
        return [pltpu.make_async_copy(out_s.at[slot, :, pl.ds(i * cw, cw)],
                                      o_hbm.at[rows, pl.ds(i * cw, cw)], sem_o.at[slot, i])
                for i in range(_OP)]

    def layernorm(r):
        rows = pl.ds(pl.multiple_of(r * _BM, _BM), _BM)
        x = ld(x_s, rows).astype(_F32)
        mean = jnp.mean(x, axis=-1, keepdims=True)
        xc = x - mean
        var = jnp.mean(xc * xc, axis=-1, keepdims=True)
        xn = (xc * jax.lax.rsqrt(var + 1e-5)).astype(_BF16)
        xn_s[pl.ds(pl.multiple_of(r * (_BM // 2), 8), _BM // 2), :] = pltpu.bitcast(xn, _U32)

    def ffn_chunk(xn, c0, cn, wait=lambda i: None):
        cols = pl.ds(c0, cn)
        wait(0)
        g = jnp.dot(xn, ld(w1_s, pl.ds(0, D), cols), preferred_element_type=_F32)
        wait(1)
        u = jnp.dot(xn, ld(w3_s, pl.ds(0, D), cols), preferred_element_type=_F32)
        h = (_silu(g) * u).astype(_BF16)
        wait(2)
        return jnp.dot(h, ld(w2_s, cols), preferred_element_type=_F32)

    K, V, Q, O = 0, 1, 2, 3

    def prologue():
        wf = [c for i, (c0, cn) in enumerate(first)
              for c in ffn_copies(pl.ds(c0, cn), sem_f, 3 * i)]
        last = len(wf) - 1
        x_copy(0).start()
        for c in wf[:last] + [x_copy(1)] + wf[last:]:
            c.start()
        for r in range(2, NB):
            x_copy(r).start()
        for c in w_copies_rest():
            c.start()
        att_s[pl.ds(0, 2), :, pl.ds(0, _HALO), :] = jnp.zeros((2, 8, _HALO, 128), _F32)
        x_copy(0).wait()
        layernorm(0)
        rows = pl.ds(0, _BM)

        def wait(n):
            wf[n].wait()
            if n == last:
                x_copy(1).wait()
                layernorm(1)

        for i, (c0, cn) in enumerate(first):
            d = ffn_chunk(ld(xn_s, rows), c0, cn, lambda k, i=i: wait(3 * i + k))
            acc_s[rows, :] = d if i == 0 else acc_s[rows, :] + d

    prologue()

    @pl.loop(1, NB)
    def _(step):
        nxt = jnp.minimum(step + 1, NB - 1)

        @pl.when(step + 1 < NB)
        def _():
            x_copy(nxt).wait()

        rows = pl.ds(pl.multiple_of(step * _BM, _BM), _BM)
        xn = ld(xn_s, rows)
        layernorm(nxt)
        acc_s[rows, :] = ffn_chunk(xn, 0, _F0)

    for c in w_copies_rest():
        c.wait()

    @pl.loop(0, NB)
    def _(blk):
        slot = blk % 2

        @pl.when(blk >= 2)
        def _():
            for c in out_copies(blk - 2, slot):
                c.wait()

        rows = pl.ds(pl.multiple_of(blk * _BM, _BM), _BM)
        xn = ld(xn_s, rows)
        lane = jax.lax.broadcasted_iota(jnp.int32, (_RG, 128), 1)
        scale = (D // _H) ** -0.5
        log2e = math.log2(math.e)

        for src, dst in ((1, K), (2, V), (0, Q)):
            y = jnp.dot(xn, ld(wqkv_s, pl.ds(0, D), pl.ds(src * D, D)),
                        preferred_element_type=_F32)
            if dst == Q:
                y = y * (scale * log2e)
            for g in range(_BM // _RG):
                yg = y[g * _RG:(g + 1) * _RG, :]
                blocks = _lane_exchange(
                    [yg[:, j * 128:(j + 1) * 128] for j in range(8)], lane)
                for j in range(8):
                    att_s[dst, j, pl.ds(_HALO + g * _RG, _RG), :] = blocks[j]

        acc = acc_s[rows, :]
        for c0 in range(_F0, F, _FC):
            acc = acc + ffn_chunk(xn, c0, _FC)

        zero = pl.multiple_of(jnp.minimum(blk, 0), 8)

        def gate(val):
            att_s[O, 0, pl.ds(zero + _BM, 8), :] = val[:8]

        def attend(g):
            r0 = _HALO + g * _RG
            masked = g * _RG < (_W - 1) * _DIL
            if masked:
                def grow():
                    return (jax.lax.broadcasted_iota(jnp.int32, (_RG, 128), 0)
                            + (blk * _BM + g * _RG))

            qs = [att_s[Q, j, pl.ds(r0, _RG), :] for j in range(8)]
            logits = []
            for w in range(_W):
                kr = pl.ds(r0 - _DIL * w, _RG)
                logits.append(functools.reduce(
                    jnp.add, [qs[j] * att_s[K, j, kr, :] for j in range(8)]))
                if w in _GATE_W:
                    gate(logits[w])
            for w in range(_W):
                l = _xor_add(_xor_add(logits[w], lane, 16), lane, 1)
                if masked and w > 0:
                    l = jnp.where(grow() >= _DIL * w, l, _NEG * log2e)
                logits[w] = l
            m = functools.reduce(jnp.maximum, logits)
            e = [jnp.exp2(l - m) for l in logits]
            inv = pl.reciprocal(functools.reduce(jnp.add, e), approx=True)

            ob = []
            for j in range(8):
                if masked:
                    v0 = jnp.broadcast_to(att_s[V, j, pl.ds(_HALO, 1), :], (_RG, 128))
                oj = None
                for w in range(_W):
                    vw = att_s[V, j, pl.ds(r0 - _DIL * w, _RG), :]
                    if masked and w > 0:
                        vw = jnp.where(grow() >= _DIL * w, vw, v0)
                    t = e[w] * vw
                    oj = t if oj is None else oj + t
                oj = oj * inv
                if j in _GATE_J:
                    gate(oj)
                ob.append(oj)
            return _lane_exchange(ob, lane)

        for g in range(_BM // _RG):
            ob = attend(g)
            for j in range(8):
                att_s[O, j, pl.ds(zero + g * _RG, _RG), :] = ob[j]
        o = jnp.concatenate(
            [att_s[O, j, pl.ds(0, _BM), :] for j in range(8)], axis=1).astype(_BF16)

        for t in (K, V):
            att_s[t, :, pl.ds(0, _HALO), :] = att_s[t, :, pl.ds(_BM, _HALO), :]

        s = jnp.dot(o, ld(wo_s, pl.ds(0, D)), preferred_element_type=_F32)

        res = (ld(x_s, rows).astype(_F32) + s * _silu(acc)).astype(_BF16)
        cw = D // _OP
        for i, c in enumerate(out_copies(blk, slot)):
            out_s[slot, :, pl.ds(i * cw, cw)] = res[:, i * cw:(i + 1) * cw]
            c.start()

    for c in out_copies(NB - 2, (NB - 2) % 2) + out_copies(NB - 1, (NB - 1) % 2):
        c.wait()


@jax.jit
def pallas_recurrent_scan__sliding_local_dilated__glu_gated_swiglu__prompt_kernel(
    A_x: jax.Array,
    A_wqkv: jax.Array,
    A_wo: jax.Array,
    B_x: jax.Array,
    B_w1: jax.Array,
    B_w3: jax.Array,
    B_w2: jax.Array,
):
    del B_x
    B, S, D = A_x.shape
    F = B_w1.shape[1]
    assert B == 1 and D == 1024 and S % _BM == 0 and S >= 2 * _BM
    assert all(a.dtype == _BF16 for a in (A_x, A_wqkv, A_wo, B_w1, B_w3, B_w2))
    NB = S // _BM

    def packed(rows, cols):
        return pltpu.VMEM((rows // 2, cols), _U32)

    any_spec = pl.BlockSpec(memory_space=pl.ANY)
    out = pl.pallas_call(
        functools.partial(_kernel, S=S, D=D, F=F),
        in_specs=[any_spec] * 6,
        out_specs=any_spec,
        out_shape=jax.ShapeDtypeStruct((S, D), A_x.dtype),
        scratch_shapes=[
            packed(S, D),
            packed(S, D),
            pltpu.VMEM((S, D), _F32),
            packed(D, 3 * D),
            packed(D, D),
            packed(D, F),
            packed(D, F),
            packed(F, D),
            pltpu.VMEM((4, 8, _HALO + _BM, 128), _F32),
            pltpu.VMEM((2, _BM, D), _BF16),
            pltpu.SemaphoreType.DMA((NB,)),
            pltpu.SemaphoreType.DMA((5,)),
            pltpu.SemaphoreType.DMA((3 * len(_FIRST),)),
            pltpu.SemaphoreType.DMA((2, _OP)),
        ],
        compiler_params=pltpu.CompilerParams(
            vmem_limit_bytes=100 * 1024 * 1024,
            flags={"XLA_TPU_EVENLY_DISTRIBUTE_CRITICAL_NODES": True},
        ),
    )(A_x.reshape(S, D), A_wqkv, A_wo, B_w1, B_w3, B_w2)
    return out.reshape(B, S, D)
```

```python
import functools
import math

import jax
import jax.numpy as jnp
import jax.experimental.pallas as pl
import jax.experimental.pallas.tpu as pltpu

_H = 32
_W = 8
_DIL = 2
_NEG = -1e9
_HALO = 16
_BM = 256
_RG = 16
_F0 = 896
_FIRST = (256, 256, 384)
_FC = 896
_OP = 4
_GATE_W = (1, 5)
_GATE_J = (1, 5)

_F32, _BF16, _U32 = jnp.float32, jnp.bfloat16, jnp.uint32


def _silu(x):
    return x * pl.reciprocal(1.0 + jnp.exp(-x), approx=True)


def _lane_exchange(blocks, lane):
    blocks = list(blocks)
    for b in range(3):
        sh = 2 << b
        m = (lane & sh) != 0
        for i in range(8):
            if i & (1 << b):
                continue
            lo, hi = blocks[i], blocks[i | (1 << b)]
            blocks[i] = jnp.where(m, pltpu.roll(hi, sh, 1), lo)
            blocks[i | (1 << b)] = jnp.where(m, hi, pltpu.roll(lo, 128 - sh, 1))
    return blocks


def _xor_add(x, lane, sh):
    m = (lane & sh) != 0
    return x + jnp.where(m, pltpu.roll(x, sh, 1), pltpu.roll(x, 128 - sh, 1))


def _kernel(x_hbm, wqkv_hbm, wo_hbm, w1_hbm, w3_hbm, w2_hbm, o_hbm,
            x_s, xn_s, acc_s, wqkv_s, wo_s, w1_s, w3_s, w2_s, att_s, out_s,
            sem_x, sem_w, sem_f, sem_o, *, S, D, F):
    NB = S // _BM

    def b16(ref):
        return ref.bitcast(_BF16)

    def ld(ref, rows, cols=slice(None)):
        if isinstance(rows.start, int):
            start = rows.start // 2
        else:
            start = pl.multiple_of(rows.start // 2, 8)
        return pltpu.bitcast(ref[pl.ds(start, rows.size // 2), cols], _BF16)

    def x_copy(r):
        rows = pl.ds(r * _BM, _BM)
        return pltpu.make_async_copy(x_hbm.at[rows, :], b16(x_s).at[rows, :], sem_x.at[r])

    def ffn_copies(cols, sem, i):
        return [
            pltpu.make_async_copy(w1_hbm.at[:, cols], b16(w1_s).at[:, cols], sem.at[i]),
            pltpu.make_async_copy(w3_hbm.at[:, cols], b16(w3_s).at[:, cols], sem.at[i + 1]),
            pltpu.make_async_copy(w2_hbm.at[cols, :], b16(w2_s).at[cols, :], sem.at[i + 2]),
        ]

    first = [(sum(_FIRST[:i]), n) for i, n in enumerate(_FIRST)]
    assert sum(_FIRST) == _F0 and (F - _F0) % _FC == 0

    def w_copies_rest():
        return ([pltpu.make_async_copy(wqkv_hbm, b16(wqkv_s), sem_w.at[0])]
                + ffn_copies(pl.ds(_F0, F - _F0), sem_w, 1)
                + [pltpu.make_async_copy(wo_hbm, b16(wo_s), sem_w.at[4])])

    def out_copies(blk, slot):
        rows = pl.ds(pl.multiple_of(blk * _BM, _BM), _BM)
        cw = D // _OP
        return [pltpu.make_async_copy(out_s.at[slot, :, pl.ds(i * cw, cw)],
                                      o_hbm.at[rows, pl.ds(i * cw, cw)], sem_o.at[slot])
                for i in range(_OP)]

    def out_wait(blk, slot):
        rows = pl.ds(pl.multiple_of(blk * _BM, _BM), _BM)
        pltpu.make_async_copy(out_s.at[slot], o_hbm.at[rows, :], sem_o.at[slot]).wait()

    def layernorm(r):
        rows = pl.ds(pl.multiple_of(r * _BM, _BM), _BM)
        x = ld(x_s, rows).astype(_F32)
        mean = jnp.mean(x, axis=-1, keepdims=True)
        xc = x - mean
        var = jnp.mean(xc * xc, axis=-1, keepdims=True)
        xn = (xc * jax.lax.rsqrt(var + 1e-5)).astype(_BF16)
        xn_s[pl.ds(pl.multiple_of(r * (_BM // 2), 8), _BM // 2), :] = pltpu.bitcast(xn, _U32)

    def ffn_chunk(xn, c0, cn, wait=lambda i: None):
        cols = pl.ds(c0, cn)
        wait(0)
        g = jnp.dot(xn, ld(w1_s, pl.ds(0, D), cols), preferred_element_type=_F32)
        wait(1)
        u = jnp.dot(xn, ld(w3_s, pl.ds(0, D), cols), preferred_element_type=_F32)
        h = (_silu(g) * u).astype(_BF16)
        wait(2)
        return jnp.dot(h, ld(w2_s, cols), preferred_element_type=_F32)

    K, V, Q, O = 0, 1, 2, 3

    def prologue():
        wf = [c for i, (c0, cn) in enumerate(first)
              for c in ffn_copies(pl.ds(c0, cn), sem_f, 3 * i)]
        last = len(wf) - 1
        x_copy(0).start()
        for c in wf[:last] + [x_copy(1)] + wf[last:]:
            c.start()
        for r in range(2, NB):
            x_copy(r).start()
        for c in w_copies_rest():
            c.start()
        att_s[pl.ds(0, 2), :, pl.ds(0, _HALO), :] = jnp.zeros((2, 8, _HALO, 128), _F32)
        x_copy(0).wait()
        layernorm(0)
        rows = pl.ds(0, _BM)

        def wait(n):
            wf[n].wait()
            if n == last:
                x_copy(1).wait()
                layernorm(1)

        for i, (c0, cn) in enumerate(first):
            d = ffn_chunk(ld(xn_s, rows), c0, cn, lambda k, i=i: wait(3 * i + k))
            acc_s[rows, :] = d if i == 0 else acc_s[rows, :] + d

    prologue()

    @pl.loop(1, NB)
    def _(step):
        nxt = jnp.minimum(step + 1, NB - 1)

        @pl.when(step + 1 < NB)
        def _():
            x_copy(nxt).wait()

        rows = pl.ds(pl.multiple_of(step * _BM, _BM), _BM)
        xn = ld(xn_s, rows)
        layernorm(nxt)
        acc_s[rows, :] = ffn_chunk(xn, 0, _F0)

    for c in w_copies_rest():
        c.wait()

    @pl.loop(0, NB)
    def _(blk):
        slot = blk % 2

        @pl.when(blk >= 2)
        def _():
            out_wait(blk - 2, slot)

        rows = pl.ds(pl.multiple_of(blk * _BM, _BM), _BM)
        xn = ld(xn_s, rows)
        lane = jax.lax.broadcasted_iota(jnp.int32, (_RG, 128), 1)
        scale = (D // _H) ** -0.5
        log2e = math.log2(math.e)

        for src, dst in ((1, K), (2, V), (0, Q)):
            y = jnp.dot(xn, ld(wqkv_s, pl.ds(0, D), pl.ds(src * D, D)),
                        preferred_element_type=_F32)
            if dst == Q:
                y = y * (scale * log2e)
            for g in range(_BM // _RG):
                yg = y[g * _RG:(g + 1) * _RG, :]
                blocks = _lane_exchange(
                    [yg[:, j * 128:(j + 1) * 128] for j in range(8)], lane)
                for j in range(8):
                    att_s[dst, j, pl.ds(_HALO + g * _RG, _RG), :] = blocks[j]

        acc = acc_s[rows, :]
        for c0 in range(_F0, F, _FC):
            acc = acc + ffn_chunk(xn, c0, _FC)

        zero = pl.multiple_of(jnp.minimum(blk, 0), 8)

        def gate(val):
            att_s[O, 0, pl.ds(zero + _BM, 8), :] = val[:8]

        def attend(g):
            r0 = _HALO + g * _RG
            masked = g * _RG < (_W - 1) * _DIL
            if masked:
                def grow():
                    return (jax.lax.broadcasted_iota(jnp.int32, (_RG, 128), 0)
                            + (blk * _BM + g * _RG))

            qs = [att_s[Q, j, pl.ds(r0, _RG), :] for j in range(8)]
            logits = []
            for w in range(_W):
                kr = pl.ds(r0 - _DIL * w, _RG)
                logits.append(functools.reduce(
                    jnp.add, [qs[j] * att_s[K, j, kr, :] for j in range(8)]))
                if w in _GATE_W:
                    gate(logits[w])
            for w in range(_W):
                l = _xor_add(_xor_add(logits[w], lane, 16), lane, 1)
                if masked and w > 0:
                    l = jnp.where(grow() >= _DIL * w, l, _NEG * log2e)
                logits[w] = l
            m = functools.reduce(jnp.maximum, logits)
            e = [jnp.exp2(l - m) for l in logits]
            inv = pl.reciprocal(functools.reduce(jnp.add, e), approx=True)

            ob = []
            for j in range(8):
                if masked:
                    v0 = jnp.broadcast_to(att_s[V, j, pl.ds(_HALO, 1), :], (_RG, 128))
                oj = None
                for w in range(_W):
                    vw = att_s[V, j, pl.ds(r0 - _DIL * w, _RG), :]
                    if masked and w > 0:
                        vw = jnp.where(grow() >= _DIL * w, vw, v0)
                    t = e[w] * vw
                    oj = t if oj is None else oj + t
                oj = oj * inv
                if j in _GATE_J:
                    gate(oj)
                ob.append(oj)
            return _lane_exchange(ob, lane)

        for g in range(_BM // _RG):
            ob = attend(g)
            for j in range(8):
                att_s[O, j, pl.ds(zero + g * _RG, _RG), :] = ob[j]
        o = jnp.concatenate(
            [att_s[O, j, pl.ds(0, _BM), :] for j in range(8)], axis=1).astype(_BF16)

        for t in (K, V):
            att_s[t, :, pl.ds(0, _HALO), :] = att_s[t, :, pl.ds(_BM, _HALO), :]

        s = jnp.dot(o, ld(wo_s, pl.ds(0, D)), preferred_element_type=_F32)

        res = (ld(x_s, rows).astype(_F32) + s * _silu(acc)).astype(_BF16)
        cw = D // _OP
        for i, c in enumerate(out_copies(blk, slot)):
            out_s[slot, :, pl.ds(i * cw, cw)] = res[:, i * cw:(i + 1) * cw]
            c.start()

    out_wait(NB - 2, (NB - 2) % 2)
    out_wait(NB - 1, (NB - 1) % 2)


@jax.jit
def pallas_recurrent_scan__sliding_local_dilated__glu_gated_swiglu__prompt_kernel(
    A_x: jax.Array,
    A_wqkv: jax.Array,
    A_wo: jax.Array,
    B_x: jax.Array,
    B_w1: jax.Array,
    B_w3: jax.Array,
    B_w2: jax.Array,
):
    del B_x
    B, S, D = A_x.shape
    F = B_w1.shape[1]
    assert B == 1 and D == 1024 and S % _BM == 0 and S >= 2 * _BM
    assert all(a.dtype == _BF16 for a in (A_x, A_wqkv, A_wo, B_w1, B_w3, B_w2))
    NB = S // _BM

    def packed(rows, cols):
        return pltpu.VMEM((rows // 2, cols), _U32)

    any_spec = pl.BlockSpec(memory_space=pl.ANY)
    out = pl.pallas_call(
        functools.partial(_kernel, S=S, D=D, F=F),
        in_specs=[any_spec] * 6,
        out_specs=any_spec,
        out_shape=jax.ShapeDtypeStruct((S, D), A_x.dtype),
        scratch_shapes=[
            packed(S, D),
            packed(S, D),
            pltpu.VMEM((S, D), _F32),
            packed(D, 3 * D),
            packed(D, D),
            packed(D, F),
            packed(D, F),
            packed(F, D),
            pltpu.VMEM((4, 8, _HALO + _BM, 128), _F32),
            pltpu.VMEM((2, _BM, D), _BF16),
            pltpu.SemaphoreType.DMA((NB,)),
            pltpu.SemaphoreType.DMA((5,)),
            pltpu.SemaphoreType.DMA((3 * len(_FIRST),)),
            pltpu.SemaphoreType.DMA((2,)),
        ],
        compiler_params=pltpu.CompilerParams(
            vmem_limit_bytes=100 * 1024 * 1024,
            flags={"XLA_TPU_EVENLY_DISTRIBUTE_CRITICAL_NODES": True},
        ),
    )(A_x.reshape(S, D), A_wqkv, A_wo, B_w1, B_w3, B_w2)
    return out.reshape(B, S, D)
```

```python
import functools
import math

import jax
import jax.numpy as jnp
import jax.experimental.pallas as pl
import jax.experimental.pallas.tpu as pltpu

_H = 32
_W = 8
_DIL = 2
_NEG = -1e9
_HALO = 16
_BM = 256
_RG = 16
_F0 = 896
_FIRST = (256, 256, 384)
_FC = 896
_AHEAD = 3
_OP = 4
_GATE_W = (1, 5)
_GATE_J = (1, 5)

_F32, _BF16, _U32 = jnp.float32, jnp.bfloat16, jnp.uint32


def _silu(x):
    return x * pl.reciprocal(1.0 + jnp.exp(-x), approx=True)


def _lane_exchange(blocks, lane):
    blocks = list(blocks)
    for b in range(3):
        sh = 2 << b
        m = (lane & sh) != 0
        for i in range(8):
            if i & (1 << b):
                continue
            lo, hi = blocks[i], blocks[i | (1 << b)]
            blocks[i] = jnp.where(m, pltpu.roll(hi, sh, 1), lo)
            blocks[i | (1 << b)] = jnp.where(m, hi, pltpu.roll(lo, 128 - sh, 1))
    return blocks


def _xor_add(x, lane, sh):
    m = (lane & sh) != 0
    return x + jnp.where(m, pltpu.roll(x, sh, 1), pltpu.roll(x, 128 - sh, 1))


def _kernel(x_hbm, wqkv_hbm, wo_hbm, w1_hbm, w3_hbm, w2_hbm, o_hbm,
            x_s, xn_s, acc_s, wqkv_s, wo_s, w1_s, w3_s, w2_s, att_s, out_s,
            sem_x, sem_w, sem_f, sem_o, *, S, D, F):
    NB = S // _BM

    def half(r):
        return pl.ds(pl.multiple_of(r * (_BM // 2), 8), _BM // 2)

    def load_xn(r):
        return pltpu.bitcast(xn_s[half(r), :], _BF16)

    def x_copy(r):
        rows = pl.ds(r * _BM, _BM)
        return pltpu.make_async_copy(x_hbm.at[rows, :], x_s.at[rows, :], sem_x.at[r])

    def ffn_copies(cols, sem, i):
        return [
            pltpu.make_async_copy(w1_hbm.at[:, cols], w1_s.at[:, cols], sem.at[i]),
            pltpu.make_async_copy(w3_hbm.at[:, cols], w3_s.at[:, cols], sem.at[i + 1]),
            pltpu.make_async_copy(w2_hbm.at[cols, :], w2_s.at[cols, :], sem.at[i + 2]),
        ]

    first = [(sum(_FIRST[:i]), n) for i, n in enumerate(_FIRST)]
    assert sum(_FIRST) == _F0

    def w_copies_rest():
        return ([pltpu.make_async_copy(wqkv_hbm, wqkv_s, sem_w.at[0])]
                + ffn_copies(pl.ds(_F0, F - _F0), sem_w, 1)
                + [pltpu.make_async_copy(wo_hbm, wo_s, sem_w.at[4])])

    def out_copies(blk, slot):
        rows = pl.ds(pl.multiple_of(blk * _BM, _BM), _BM)
        cw = D // _OP
        return [pltpu.make_async_copy(out_s.at[slot, :, pl.ds(i * cw, cw)],
                                      o_hbm.at[rows, pl.ds(i * cw, cw)], sem_o.at[slot])
                for i in range(_OP)]

    def out_wait(blk, slot):
        rows = pl.ds(pl.multiple_of(blk * _BM, _BM), _BM)
        pltpu.make_async_copy(out_s.at[slot], o_hbm.at[rows, :], sem_o.at[slot]).wait()

    def layernorm(r):
        rows = pl.ds(pl.multiple_of(r * _BM, _BM), _BM)
        x = x_s[rows, :].astype(_F32)
        mean = jnp.mean(x, axis=-1, keepdims=True)
        xc = x - mean
        var = jnp.mean(xc * xc, axis=-1, keepdims=True)
        xn = (xc * jax.lax.rsqrt(var + 1e-5)).astype(_BF16)
        xn_s[half(r), :] = pltpu.bitcast(xn, _U32)

    def ffn_chunk(xn, c0, cn, wait=lambda i: None):
        cols = pl.ds(c0, cn)
        wait(0)
        g = jnp.dot(xn, w1_s[:, cols], preferred_element_type=_F32)
        wait(1)
        u = jnp.dot(xn, w3_s[:, cols], preferred_element_type=_F32)
        h = (_silu(g) * u).astype(_BF16)
        wait(2)
        return jnp.dot(h, w2_s[cols, :], preferred_element_type=_F32)

    K, V, Q, O = 0, 1, 2, 3

    def prologue():
        wf = [c for i, (c0, cn) in enumerate(first)
              for c in ffn_copies(pl.ds(c0, cn), sem_f, 3 * i)]
        last = len(wf) - 1
        order = wf[:last] + [x_copy(1)] + wf[last:]
        later = [x_copy(r) for r in range(2, NB)]
        x_copy(0).start()
        order[0].start()
        att_s[pl.ds(0, 2), :, pl.ds(0, _HALO), :] = jnp.zeros((2, 8, _HALO, 128), _F32)
        x_copy(0).wait()
        for c in order[1:_AHEAD]:
            c.start()
        layernorm(0)
        rows = pl.ds(0, _BM)

        def wait(n):
            wf[n].wait()
            pos = n if n < last else last + 1
            for c in order[pos + _AHEAD:pos + _AHEAD + (2 if n == last - 1 else 1)]:
                c.start()
            if n == last:
                for c in later:
                    c.start()
                x_copy(1).wait()
                layernorm(1)

        for i, (c0, cn) in enumerate(first):
            d = ffn_chunk(load_xn(0), c0, cn, lambda k, i=i: wait(3 * i + k))
            acc_s[rows, :] = d if i == 0 else acc_s[rows, :] + d

    prologue()

    @pl.loop(1, NB)
    def _(step):
        nxt = jnp.minimum(step + 1, NB - 1)

        for i, c in enumerate(w_copies_rest()):
            pl.when(step == i + 1)(c.start)

        @pl.when(step + 1 < NB)
        def _():
            x_copy(nxt).wait()

        rows = pl.ds(pl.multiple_of(step * _BM, _BM), _BM)
        xn = load_xn(step)
        layernorm(nxt)
        acc_s[rows, :] = ffn_chunk(xn, 0, _F0)

    for c in w_copies_rest():
        c.wait()

    @pl.loop(0, NB)
    def _(blk):
        slot = blk % 2

        @pl.when(blk >= 2)
        def _():
            out_wait(blk - 2, slot)

        rows = pl.ds(pl.multiple_of(blk * _BM, _BM), _BM)
        xn = load_xn(blk)
        lane = jax.lax.broadcasted_iota(jnp.int32, (_RG, 128), 1)
        scale = (D // _H) ** -0.5
        log2e = math.log2(math.e)

        for src, dst in ((1, K), (2, V), (0, Q)):
            y = jnp.dot(xn, wqkv_s[:, pl.ds(src * D, D)], preferred_element_type=_F32)
            if dst == Q:
                y = y * (scale * log2e)
            for g in range(_BM // _RG):
                yg = y[g * _RG:(g + 1) * _RG, :]
                blocks = _lane_exchange(
                    [yg[:, j * 128:(j + 1) * 128] for j in range(8)], lane)
                for j in range(8):
                    att_s[dst, j, pl.ds(_HALO + g * _RG, _RG), :] = blocks[j]

        acc = acc_s[rows, :]
        for c0 in range(_F0, F, _FC):
            acc = acc + ffn_chunk(xn, c0, min(_FC, F - c0))

        zero = pl.multiple_of(jnp.minimum(blk, 0), 8)

        def gate(val):
            att_s[O, 0, pl.ds(zero + _BM, 8), :] = val[:8]

        def attend(g):
            r0 = _HALO + g * _RG
            masked = g * _RG < (_W - 1) * _DIL
            if masked:
                def grow():
                    return (jax.lax.broadcasted_iota(jnp.int32, (_RG, 128), 0)
                            + (blk * _BM + g * _RG))

            qs = [att_s[Q, j, pl.ds(r0, _RG), :] for j in range(8)]
            logits = []
            for w in range(_W):
                kr = pl.ds(r0 - _DIL * w, _RG)
                logits.append(functools.reduce(
                    jnp.add, [qs[j] * att_s[K, j, kr, :] for j in range(8)]))
                if w in _GATE_W:
                    gate(logits[w])
            for w in range(_W):
                l = _xor_add(_xor_add(logits[w], lane, 16), lane, 1)
                if masked and w > 0:
                    l = jnp.where(grow() >= _DIL * w, l, _NEG * log2e)
                logits[w] = l
            m = functools.reduce(jnp.maximum, logits)
            e = [jnp.exp2(l - m) for l in logits]
            inv = pl.reciprocal(functools.reduce(jnp.add, e), approx=True)

            ob = []
            for j in range(8):
                if masked:
                    v0 = jnp.broadcast_to(att_s[V, j, pl.ds(_HALO, 1), :], (_RG, 128))
                oj = None
                for w in range(_W):
                    vw = att_s[V, j, pl.ds(r0 - _DIL * w, _RG), :]
                    if masked and w > 0:
                        vw = jnp.where(grow() >= _DIL * w, vw, v0)
                    t = e[w] * vw
                    oj = t if oj is None else oj + t
                oj = oj * inv
                if j in _GATE_J:
                    gate(oj)
                ob.append(oj)
            return _lane_exchange(ob, lane)

        for g in range(_BM // _RG):
            ob = attend(g)
            for j in range(8):
                att_s[O, j, pl.ds(zero + g * _RG, _RG), :] = ob[j]
        o = jnp.concatenate(
            [att_s[O, j, pl.ds(0, _BM), :] for j in range(8)], axis=1).astype(_BF16)

        for t in (K, V):
            att_s[t, :, pl.ds(0, _HALO), :] = att_s[t, :, pl.ds(_BM, _HALO), :]

        s = jnp.dot(o, wo_s[...], preferred_element_type=_F32)

        res = (x_s[rows, :].astype(_F32) + s * _silu(acc)).astype(_BF16)
        cw = D // _OP
        for i, c in enumerate(out_copies(blk, slot)):
            out_s[slot, :, pl.ds(i * cw, cw)] = res[:, i * cw:(i + 1) * cw]
            c.start()

    out_wait(NB - 2, (NB - 2) % 2)
    out_wait(NB - 1, (NB - 1) % 2)


@jax.jit
def pallas_recurrent_scan__sliding_local_dilated__glu_gated_swiglu__prompt_kernel(
    A_x: jax.Array,
    A_wqkv: jax.Array,
    A_wo: jax.Array,
    B_x: jax.Array,
    B_w1: jax.Array,
    B_w3: jax.Array,
    B_w2: jax.Array,
):
    del B_x
    B, S, D = A_x.shape
    F = B_w1.shape[1]
    assert B == 1 and D == 1024 and S % _BM == 0 and S // _BM > 5
    assert all(a.dtype == _BF16 for a in (A_x, A_wqkv, A_wo, B_w1, B_w3, B_w2))
    NB = S // _BM

    any_spec = pl.BlockSpec(memory_space=pl.ANY)
    out = pl.pallas_call(
        functools.partial(_kernel, S=S, D=D, F=F),
        in_specs=[any_spec] * 6,
        out_specs=any_spec,
        out_shape=jax.ShapeDtypeStruct((S, D), A_x.dtype),
        scratch_shapes=[
            pltpu.VMEM((S, D), _BF16),
            pltpu.VMEM((S // 2, D), _U32),
            pltpu.VMEM((S, D), _F32),
            pltpu.VMEM((D, 3 * D), _BF16),
            pltpu.VMEM((D, D), _BF16),
            pltpu.VMEM((D, F), _BF16),
            pltpu.VMEM((D, F), _BF16),
            pltpu.VMEM((F, D), _BF16),
            pltpu.VMEM((4, 8, _HALO + _BM, 128), _F32),
            pltpu.VMEM((2, _BM, D), _BF16),
            pltpu.SemaphoreType.DMA((NB,)),
            pltpu.SemaphoreType.DMA((5,)),
            pltpu.SemaphoreType.DMA((3 * len(_FIRST),)),
            pltpu.SemaphoreType.DMA((2,)),
        ],
        compiler_params=pltpu.CompilerParams(
            vmem_limit_bytes=100 * 1024 * 1024,
            flags={"XLA_TPU_EVENLY_DISTRIBUTE_CRITICAL_NODES": True},
        ),
    )(A_x.reshape(S, D), A_wqkv, A_wo, B_w1, B_w3, B_w2)
    return out.reshape(B, S, D)
```
